```python
import os as _os
_os.environ.setdefault("JAX_PLATFORMS", "cpu")
import jax
import jax.numpy as jnp

def _softmax(x, axis=-1):
    return jax.nn.softmax(x, axis=axis)
def _gelu(x):
    return jax.nn.gelu(x, approximate=True)
def _silu(x):
    return jax.nn.silu(x)
def _sigmoid(x):
    return jax.nn.sigmoid(x)
def _layernorm(x, axis=-1, eps=1e-5):
    m = jnp.mean(x, axis=axis, keepdims=True)
    v = jnp.var(x, axis=axis, keepdims=True)
    return (x - m) / jnp.sqrt(v + eps)
def _scatter_add(tgt, idx, src, axis=0):
    return tgt.at[idx].add(src)
def _segment_sum(src, seg, n):
    return jax.ops.segment_sum(src, seg, n)
class _Rng:
    def __init__(self, key):
        self._k = key
    def _next(self):
        self._k, sub = jax.random.split(self._k)
        return sub
    def normal(self, shape):
        return jax.random.normal(self._next(), shape, dtype=jnp.bfloat16)
    def randint(self, lo, hi, shape):
        return jax.random.randint(self._next(), shape, lo, hi, dtype=jnp.int32)
    def uniform(self, shape, lo=0.0, hi=1.0):
        return jax.random.uniform(self._next(), shape, jnp.bfloat16, lo, hi)
    def permutation(self, n):
        return jax.random.permutation(self._next(), n)


kernel_name = 'interleave_layers__sliding_block_cached__mixer_channel_mlp__decode'

def setup_inputs():
    _rng = _Rng(jax.random.key(int.from_bytes(__import__("os").urandom(4), "little")))
    _w = (lambda a: (lambda t: t.astype(jnp.bfloat16) if jnp.issubdtype(t.dtype, jnp.floating) else t)(jnp.asarray(a)))
    def _A_setup():
        B, Sq, D = 8, 1, 640
        Hq, Hkv, Sk, Dh = 32, 32, 4096, 128
        assert Hq % Hkv == 0, (Hq, Hkv)
        return {
            "x": _w((lambda *s: _rng.normal(s) * 0.05)(B, Sq, D)),
            "k_cache": _w((lambda *s: _rng.normal(s) * 1.6)(B, Hkv, Sk, Dh)),
            "v_cache": _w((lambda *s: _rng.normal(s) * 0.8)(B, Hkv, Sk, Dh)),
            "wq": _w((lambda *s: _rng.normal(s) * 1.6)(D, Hq * Dh) * (D ** -0.5)),
            "wo": _w((lambda *s: _rng.normal(s) * 0.8)(Hq * Dh, D) * ((Hq * Dh) ** -0.5)),
        }
    _A_in = _A_setup()

    def _B_setup():
        B, S, D, F = 8, 1, 640, 1728
        return {
            "x": _w((lambda *s: _rng.normal(s) * 0.05)(B, S, D)),
            "w1": _w((lambda *s: _rng.normal(s) * 0.4)(D, F) * (D ** -0.5)),
            "b1": _w((lambda *s: _rng.normal(s) * 0.4)(F)),
            "w2": _w((lambda *s: _rng.normal(s) * 0.4)(F, D) * (F ** -0.5)),
            "b2": _w((lambda *s: _rng.normal(s) * 0.2)(D)),
        }
    _B_in = _B_setup()

    return {
        "A_x": _A_in["x"],
        "A_k_cache": _A_in["k_cache"],
        "A_v_cache": _A_in["v_cache"],
        "A_wq": _A_in["wq"],
        "A_wo": _A_in["wo"],
        "B_x": _B_in["x"],
        "B_w1": _B_in["w1"],
        "B_b1": _B_in["b1"],
        "B_w2": _B_in["w2"],
        "B_b2": _B_in["b2"],
    }

def reference(A_x, A_k_cache, A_v_cache, A_wq, A_wo, B_x, B_w1, B_b1, B_w2, B_b2):
    def _A_ref(x, k_cache, v_cache, wq, wo):
        B, Sq, D = x.shape
        Hq, Dh = 32, 128
        Hkv, Sk = k_cache.shape[1], k_cache.shape[2]
        W = min(4096, max(256, Sk // 4))
        rep = Hq // Hkv
        q = (lambda x, *d: x.transpose(*d))((x @ wq).reshape(B, Sq, Hq, Dh), 0, 2, 1, 3)
        k = jnp.repeat(k_cache[:, :, Sk - W:, :], rep, axis=1)
        v = jnp.repeat(v_cache[:, :, Sk - W:, :], rep, axis=1)
        scores = jnp.einsum("bhqd,bhkd->bhqk", q, k) * (Dh ** -0.5)
        p = _softmax(scores, axis=-1)
        o = jnp.einsum("bhqk,bhkd->bhqd", p, v)
        return (lambda x, *d: x.transpose(*d))(o, 0, 2, 1, 3).reshape(B, Sq, Hq * Dh) @ wo

    def _B_ref(x, w1, b1, w2, b2):
        y = _layernorm(x, axis=-1)
        h = _gelu(jnp.einsum("bsd,df->bsf", y, w1) + b1)
        return jnp.einsum("bsf,fd->bsd", h, w2) + b2

    x = A_x
    x = x + _A_ref(_layernorm(x, axis=-1), A_k_cache, A_v_cache, A_wq, A_wo)
    x = x + _B_ref(_layernorm(x, axis=-1), B_w1, B_b1, B_w2, B_b2)
    x = x + _A_ref(_layernorm(x, axis=-1), A_k_cache, A_v_cache, A_wq, A_wo)
    x = x + _B_ref(_layernorm(x, axis=-1), B_w1, B_b1, B_w2, B_b2)
    return x
```

```python
import functools
import jax
import jax.numpy as jnp
from jax import lax
from jax.experimental import pallas as pl
from jax.experimental.pallas import tpu as pltpu

NT = (((1,), (1,)), ((), ()))
F32 = jnp.float32
BF16 = jnp.bfloat16
LOG2E = 1.4426950408889634


def _layernorm(x):
    m = jnp.mean(x, axis=-1, keepdims=True)
    d = x - m
    v = jnp.mean(d * d, axis=-1, keepdims=True)
    return d * lax.rsqrt(v + 1e-5)


def _gelu(x):
    c = 0.7978845608028654
    return 0.5 * x * (1.0 + jnp.tanh(c * (x + 0.044715 * (x * x * x))))


def make(HG=4, ROWS=32, TAILG=8):
    def run(A_x, A_k_cache, A_v_cache, A_wq, A_wo, B_x, B_w1, B_b1, B_w2, B_b2):
        B, _, D = A_x.shape
        _, H, SK, DH = A_k_cache.shape
        W = min(4096, max(256, SK // 4))
        F = B_w1.shape[1]
        NG = H // HG
        scale2 = (DH ** -0.5) * LOG2E

        def kern(x_hbm, k_hbm, v_hbm, wq_hbm, wo_hbm, w1t_hbm, b1_hbm, w2_hbm, b2_hbm, o_hbm,
                 kbuf, vbuf, wq_v, wo_v, w1t_v, w2_v, x_v, b1_v, b2_v, xs, qs, acc, out_v,
                 kv_sem, w_sem):

            def start_kv(bh, slot, h0):
                for s0 in range(0, W, ROWS):
                    pltpu.make_async_copy(
                        k_hbm.at[pl.ds(bh, HG), pl.ds(SK - W + s0, ROWS), :],
                        kbuf.at[slot, pl.ds(h0, HG), pl.ds(s0, ROWS), :],
                        kv_sem.at[slot, h0 // HG]).start(priority=0)
                    pltpu.make_async_copy(
                        v_hbm.at[pl.ds(bh, HG), pl.ds(SK - W + s0, ROWS), :],
                        vbuf.at[slot, pl.ds(h0, HG), pl.ds(s0, ROWS), :],
                        kv_sem.at[slot, h0 // HG]).start(priority=1)

            def wait_kv(slot, h0):
                kb = kbuf.at[slot, pl.ds(h0, HG)]
                vb = vbuf.at[slot, pl.ds(h0, HG)]
                pltpu.make_async_copy(kb, kb, kv_sem.at[slot, h0 // HG]).wait()
                pltpu.make_async_copy(vb, vb, kv_sem.at[slot, h0 // HG]).wait()

            def start_w(src, dst, sem, rows, cols):
                R, C = src.shape
                i = 0
                chunks = [(r, c) for r in range(0, R, rows) for c in range(0, C, cols)]
                n = len(chunks)
                half = (n + 1) // 2
                for a in range(half):
                    for p, idx in ((0, a), (1, a + half)):
                        if idx < n:
                            r, c = chunks[idx]
                            pltpu.make_async_copy(src.at[pl.ds(r, rows), pl.ds(c, cols)],
                                                  dst.at[pl.ds(r, rows), pl.ds(c, cols)], sem).start(priority=p)

            def wait_all(dst, sem):
                pltpu.make_async_copy(dst, dst, sem).wait()

            cx = pltpu.make_async_copy(x_hbm, x_v, w_sem.at[0]); cx.start()
            start_w(wq_hbm, wq_v, w_sem.at[3], 32, 512)
            cb1 = pltpu.make_async_copy(b1_hbm, b1_v, w_sem.at[1]); cb1.start()
            cb2 = pltpu.make_async_copy(b2_hbm, b2_v, w_sem.at[2]); cb2.start()
            start_kv(0, 0, 0)
            cx.wait()
            x0 = x_v[...].astype(F32)
            xs[...] = x0
            acc[...] = jnp.zeros_like(acc)
            wait_all(wq_v, w_sem.at[3])
            qs[...] = jnp.dot(_layernorm(x0).astype(BF16), wq_v[...], preferred_element_type=F32)
            start_w(wo_hbm, wo_v, w_sem.at[4], 32, 640)
            start_w(w1t_hbm, w1t_v, w_sem.at[5], 32, 640)
            start_w(w2_hbm, w2_v, w_sem.at[6], 32, 640)
            cb1.wait(); cb2.wait()
            wait_all(wo_v, w_sem.at[4])

            row_w = lax.broadcasted_iota(jnp.int32, (B, W), 0)
            row_d = lax.broadcasted_iota(jnp.int32, (B, DH), 0)
            row_x = lax.broadcasted_iota(jnp.int32, (B, D), 0)

            def attend(h0, nh, srcs):
                ps, ls = [], []
                for j in range(nh):
                    c0 = pl.multiple_of((h0 + j) * DH, DH)
                    q = qs[:, pl.ds(c0, DH)].astype(BF16)
                    S = None
                    for r, slot in srcs:
                        s = lax.dot_general(q, kbuf[slot, h0 + j], NT, preferred_element_type=F32)
                        S = s if S is None else jnp.where(row_w == r, s, S)
                    m = jnp.max(S, axis=-1, keepdims=True)
                    p = jnp.exp2((S - m) * scale2)
                    ls.append(jnp.sum(p, axis=-1, keepdims=True))
                    ps.append(p.astype(BF16))
                os_ = []
                for j in range(nh):
                    O = None
                    for r, slot in srcs:
                        o = jnp.dot(ps[j], vbuf[slot, h0 + j], preferred_element_type=F32)
                        O = o if O is None else jnp.where(row_d == r, o, O)
                    os_.append((O / ls[j]).astype(BF16))
                A = jnp.concatenate(os_, axis=-1)
                r0 = pl.multiple_of(h0 * DH, nh * DH)
                acc[...] += jnp.dot(A, wo_v[pl.ds(r0, nh * DH), :], preferred_element_type=F32)

            def mlp(active):
                x1 = xs[...] + acc[...]
                y = _layernorm(x1).astype(BF16)
                b1 = b1_v[...].astype(F32).reshape(1, F)
                b2 = b2_v[...].astype(F32).reshape(1, D)
                h = _gelu(lax.dot_general(y, w1t_v[...], NT, preferred_element_type=F32) + b1)
                x2 = x1 + jnp.dot(h.astype(BF16), w2_v[...], preferred_element_type=F32) + b2
                xn = jnp.where(active, x2, xs[...])
                xs[...] = xn
                acc[...] = jnp.zeros_like(acc)
                return xn

            def qproj(xn):
                qs[...] = jnp.dot(_layernorm(xn).astype(BF16), wq_v[...], preferred_element_type=F32)

            def g0(g, c):
                nxt = g + 1
                start_kv(nxt * HG, nxt // NG, (nxt % NG) * HG)
                wait_kv(0, g * HG)
                attend(g * HG, HG, [(0, 0)])
                return c
            lax.fori_loop(0, NG, g0, 0)
            wait_all(w1t_v, w_sem.at[5]); wait_all(w2_v, w_sem.at[6])
            qproj(mlp(row_x == 0))

            def step(s, c):
                slot = s % 2
                def gbody(g, c):
                    nxt = s * NG + g + 1
                    @pl.when(nxt < B * NG)
                    def _():
                        start_kv(nxt * HG, (nxt // NG) % 2, (nxt % NG) * HG)
                    wait_kv(slot, g * HG)
                    attend(g * HG, HG, [(s - 1, 1 - slot), (s, slot)])
                    return c
                lax.fori_loop(0, NG, gbody, 0)
                qproj(mlp((row_x == s) | (row_x == s - 1)))
                return c
            lax.fori_loop(1, B, step, 0)

            def tbody(g, c):
                attend(g * TAILG, TAILG, [(B - 1, (B - 1) % 2)])
                return c
            lax.fori_loop(0, H // TAILG, tbody, 0)
            xn = mlp(row_x == B - 1)
            out_v[...] = xn.astype(out_v.dtype)
            co = pltpu.make_async_copy(out_v, o_hbm, w_sem.at[0]); co.start(); co.wait()

        hbm = pl.BlockSpec(memory_space=pltpu.HBM)
        out = pl.pallas_call(
            kern,
            out_shape=jax.ShapeDtypeStruct((B, D), A_x.dtype),
            in_specs=[hbm] * 9,
            out_specs=hbm,
            scratch_shapes=[
                pltpu.VMEM((2, H, W, DH), BF16), pltpu.VMEM((2, H, W, DH), BF16),
                pltpu.VMEM((D, H * DH), BF16), pltpu.VMEM((H * DH, D), BF16),
                pltpu.VMEM((F, D), BF16), pltpu.VMEM((F, D), BF16),
                pltpu.VMEM((B, D), BF16), pltpu.VMEM((F,), BF16), pltpu.VMEM((D,), BF16),
                pltpu.VMEM((B, D), F32), pltpu.VMEM((B, H * DH), F32), pltpu.VMEM((B, D), F32),
                pltpu.VMEM((B, D), A_x.dtype),
                pltpu.SemaphoreType.DMA((2, NG)), pltpu.SemaphoreType.DMA((7,)),
            ],
            compiler_params=pltpu.CompilerParams(vmem_limit_bytes=100 * 2**20, disable_bounds_checks=True),
        )(A_x.reshape(B, D), A_k_cache.reshape(B * H, SK, DH), A_v_cache.reshape(B * H, SK, DH),
          A_wq, A_wo, B_w1.T, B_b1, B_w2, B_b2)
        return out.reshape(B, 1, D)
    return run


@jax.jit
def pallas_interleave_layers__sliding_block_cached__mixer_channel_mlp__decode_kernel(A_x, A_k_cache, A_v_cache, A_wq, A_wo, B_x, B_w1, B_b1, B_w2, B_b2):
    return make()(A_x, A_k_cache, A_v_cache, A_wq, A_wo, B_x, B_w1, B_b1, B_w2, B_b2)
```

```python
import contextlib
import jax
import jax.numpy as jnp
from jax import lax
from jax.experimental import pallas as pl
from jax.experimental.pallas import tpu as pltpu

NT = (((1,), (1,)), ((), ()))
F32 = jnp.float32
BF16 = jnp.bfloat16
U32 = jnp.uint32
LOG2E = 1.4426950408889634
EPS = 1e-5


def _center(x):
    d = x - jnp.mean(x, axis=-1, keepdims=True)
    return d, lax.rsqrt(jnp.mean(d * d, axis=-1, keepdims=True) + EPS)


def _layernorm(x):
    d, rs = _center(x)
    return d * rs


def _gelu(x):
    c = 0.7978845608028654
    return (0.5 * x) * (1.0 + jnp.tanh(x * (c + (c * 0.044715) * (x * x))))


def _interleave(*streams):
    pos, t = [0] * len(streams), [0.0] * len(streams)
    while True:
        live = [i for i in range(len(streams)) if pos[i] < len(streams[i])]
        if not live:
            return
        i = min(live, key=lambda i: t[i])
        cost, thunk = streams[i][pos[i]]
        thunk()
        pos[i] += 1
        t[i] += cost


def make(A1=14, DI=2, DM=3, CH=4, scopes=False, FM=1024, L=24, PE=6, NX=4, LM=0, PEM=4, NB=256, MG=4, vparts=((0, 4), (4, 2), (6, 2)), Q=116, T0=40, TG=(152, 176, 204, 253, 301, 344, 387), M6=8, nodma=False, nocomp=False, pmode=1):
    scope = jax.named_scope if scopes else (lambda n: contextlib.nullcontext())

    def run(A_x, A_k_cache, A_v_cache, A_wq, A_wo, B_x, B_w1, B_b1, B_w2, B_b2):
        B, _, D = A_x.shape
        _, H, SK, DH = A_k_cache.shape
        W = min(4096, max(256, SK // 4))
        F = B_w1.shape[1]
        E = H * DH
        FP = pl.cdiv(F, 128) * 128
        GH, PAIR, ROWS = 8, 2, 64
        NG = H // GH
        NQ, NO, NW = 5, 4, 4
        NV = 2
        HV = NV * GH
        HM = H - HV
        FV = F - FM
        TD, TW = D // 128, W // 128
        scale2 = (DH ** -0.5) * LOG2E
        NC = W // ROWS
        NP = NC * GH // PAIR
        last = B - 1
        lslot = last % 2

        def kern(x_hbm, k_hbm, v_hbm, wq_hbm, wo_hbm, w1t_hbm, b1_hbm, w2_hbm, b2_hbm, o_hbm,
                 kbuf, vbuf, wq_v, wo_v, w1t_v, w2_v, x_v, b1_v, b2_v, out_v,
                 wqu, wou, w1u, w2u, b1r, b2r, xs, qs, acc, pbuf, lbuf,
                 ktb, qk8, vo8, wox, wm, b1c,
                 kv_sem, k_sem, v_sem, w_sem):
            bc = lambda u: pltpu.bitcast(u, BF16)

            def ld(ref, *idx):
                return bc(ref.bitcast(U32)[idx])

            def kv_copy(src, dst, bh, slot, h, s, sem):
                return pltpu.make_async_copy(
                    src.at[pl.ds(bh, PAIR), pl.ds(SK - W + s, ROWS), :],
                    dst.at[slot, pl.ds(h, PAIR), pl.ds(s, ROWS), :], sem)

            def chunks(lo, hi, fn):
                if hi > lo and not nodma:
                    lax.fori_loop(lo, hi, lambda c, carry: (fn(c), carry)[1], 0)

            def start_kv(G, lo, hi):
                if isinstance(G, int):
                    slot, g = (G // NG) % 2, G % NG
                else:
                    slot, g = lax.shift_right_logical(G, NG.bit_length() - 1) & 1, G & (NG - 1)

                def chunk(c):
                    s = pl.multiple_of(c * ROWS, ROWS)
                    for h in range(0, GH, PAIR):
                        kv_copy(k_hbm, kbuf, G * GH + h, slot, g * GH + h, s, kv_sem.at[slot, g]).start(priority=0)
                        kv_copy(v_hbm, vbuf, G * GH + h, slot, g * GH + h, s, kv_sem.at[slot, g]).start(priority=1)
                chunks(lo, hi, chunk)

            def wait_heads(buf, slot, h0, n, sem):
                if nodma: return
                r = buf.at[slot, pl.ds(h0, n)]
                pltpu.make_async_copy(r, r, sem).wait()

            v_parts = [(g * GH, GH) for g in range(NG - 1)] + [((NG - 1) * GH + h, n) for h, n in vparts]
            parts = [(k_hbm, kbuf, g * GH, GH, k_sem.at[g]) for g in range(NG)]
            parts += [(v_hbm, vbuf, h0, n, v_sem.at[i]) for i, (h0, n) in enumerate(v_parts)]
            issued = [0]

            def start_last(upto):
                first = 0
                for src, dst, h0, n, sem in parts:
                    half = max(n // 2, PAIR)
                    per = 2 * half // PAIR
                    steps = n // PAIR * NC // per

                    def chunk(c, src=src, dst=dst, h0=h0, n=n, sem=sem, half=half):
                        for h in range(h0, h0 + half, PAIR):
                            s = pl.multiple_of(c * ROWS, ROWS)
                            kv_copy(src, dst, last * H + h, lslot, h, s, sem).start(priority=0)
                            if n > PAIR:
                                kv_copy(src, dst, last * H + h + half, lslot, h + half, s, sem).start(priority=1)
                            else:
                                kv_copy(src, dst, last * H + h, lslot, h, s + W // 2, sem).start(priority=1)
                    lo, hi = (min(max((e - first) // per, 0), steps) for e in (issued[0], upto))
                    chunks(lo, hi, chunk)
                    first += steps * per
                issued[0] = max(issued[0], upto)

            def start_weights(src0, dst0, sem0, cols, src1, dst1, sem1, lo, hi):
                n0, n1 = src0.shape[1] // 8, src1.shape[1] // 8
                assert n1 % n0 == 0

                def strip(c):
                    r = pl.multiple_of(c * 8, 8)
                    q0 = [pltpu.make_async_copy(src0.at[:, pl.ds(r, 8), pl.ds(c0, cols)], dst0.at[:, pl.ds(r, 8), pl.ds(c0, cols)], sem0)
                          for c0 in range(0, src0.shape[2], cols)]
                    q1 = [pltpu.make_async_copy(src1.at[:, pl.ds(r * (n1 // n0) + 8 * i, 8)], dst1.at[:, pl.ds(r * (n1 // n0) + 8 * i, 8)], sem1)
                          for i in range(n1 // n0)]
                    assert len(q0) == len(q1)
                    for a, b in zip(q0, q1):
                        a.start(priority=0)
                        b.start(priority=1)
                lax.fori_loop(lo, hi, lambda c, carry: (strip(c), carry)[1], 0)

            def wait_all(dst, sem):
                pltpu.make_async_copy(dst, dst, sem).wait()

            cx = pltpu.make_async_copy(x_hbm, x_v, w_sem.at[0])
            cb1 = pltpu.make_async_copy(b1_hbm, b1_v, w_sem.at[1])
            cb2 = pltpu.make_async_copy(b2_hbm, b2_v, w_sem.at[2])
            cx.start()
            start_weights(wq_hbm, wq_v, w_sem.at[3], 512, wo_hbm, wo_v, w_sem.at[4], 0, D // NQ // 8)
            cb1.start()
            cb2.start()
            start_weights(w1t_hbm, w1t_v, w_sem.at[5], D, w2_hbm, w2_v, w_sem.at[6], 0, F // NW // 8)
            cx.wait()
            x0 = x_v[...].astype(F32)
            xs[...] = x0
            acc[...] = jnp.zeros_like(acc)
            wait_all(wq_v, w_sem.at[3])
            wqu[...] = pltpu.bitcast(wq_v[...].reshape(D, E), U32)
            start_kv(0, 0, NC // 2)
            qs[...] = jnp.dot(_layernorm(x0).astype(BF16), bc(wqu[...]), preferred_element_type=F32)
            start_kv(0, NC // 2, NC)
            wait_all(wo_v, w_sem.at[4])
            wou[...] = pltpu.bitcast(wo_v[...].reshape(E, D), U32)
            start_kv(1, 0, A1 // 2)
            cb1.wait()
            cb2.wait()
            wait_all(w1t_v, w_sem.at[5])
            wait_all(w2_v, w_sem.at[6])
            w1t = w1t_v[...].reshape(F, D)
            for f0 in range(0, 0 if nocomp else F, 128):
                n = min(128, F - f0)
                blk = w1t[f0:f0 + n]
                if n < 128:
                    blk = jnp.concatenate([blk, jnp.zeros((128 - n, D), BF16)], axis=0)
                w1u[:, pl.ds(f0, 128)] = pltpu.bitcast(blk.T, U32)
            w2u[...] = pltpu.bitcast(w2_v[...].reshape(F, D), U32)
            b1 = b1_v[...].astype(F32).reshape(1, F)
            b1 = jnp.concatenate([b1, jnp.zeros((1, FP - F), F32)], axis=1)
            b1r[...] = jnp.broadcast_to(b1, (8, FP))
            b2r[...] = jnp.broadcast_to(b2_v[...].astype(F32).reshape(1, D), (8, D))
            start_kv(1, A1 // 2, A1)

            row_w = lax.broadcasted_iota(jnp.int32, (8, W), 0)
            row_d = lax.broadcasted_iota(jnp.int32, (8, DH), 0)
            row_x = lax.broadcasted_iota(jnp.int32, (8, D), 0)

            def lanes(i, n=1):
                return pl.ds(i * DH, n * DH) if isinstance(i, int) else pl.ds(pl.multiple_of(i * DH, DH), n * DH)

            def probs(h, srcs, kt_row=None):
                if nocomp: return jnp.zeros((8, W), BF16), jnp.zeros((8, 1), F32)
                q = qs[:, lanes(h)].astype(BF16)
                S = None
                for r, slot in srcs:
                    if r is kt_row:
                        s = jnp.dot(q, bc(ktb[h]), preferred_element_type=F32)
                    else:
                        s = lax.dot_general(q, ld(kbuf, slot, h), NT, preferred_element_type=F32)
                    S = s if S is None else jnp.where(row_w == r, s, S)
                p = jnp.exp2((S - jnp.max(S, axis=-1, keepdims=True)) * scale2)
                return p.astype(BF16), jnp.sum(p, axis=-1, keepdims=True)

            def project(h0, srcs, pls):
                if nocomp: return
                outs = []
                for j, (p, l) in enumerate(pls):
                    O = jnp.zeros((8, DH), F32)
                    for r, slot in srcs:
                        o = jnp.dot(p, ld(vbuf, slot, h0 + j), preferred_element_type=F32)
                        O = jnp.where(row_d == r, o, O)
                    outs.append((O / l).astype(BF16))
                n = len(pls) * DH // 2
                r0 = h0 * (DH // 2)
                w = wou[pl.ds(r0 if isinstance(r0, int) else pl.multiple_of(r0, DH // 2), n), :]
                acc[...] += jnp.dot(jnp.concatenate(outs, axis=-1), bc(w), preferred_element_type=F32)

            def mlp(active):
                if nocomp: return xs[...]
                x1 = xs[...] + acc[...]
                y = _layernorm(x1).astype(BF16)
                h = _gelu(jnp.dot(y, bc(w1u[...]), preferred_element_type=F32) + b1r[...])[:, :F]
                x2 = x1 + jnp.dot(h.astype(BF16), bc(w2u[...]), preferred_element_type=F32) + b2r[...]
                xn = jnp.where(active, x2, xs[...])
                xs[...] = xn
                acc[...] = jnp.where(active, 0.0, acc[...])
                return xn

            def qproj(xn):
                if nocomp: return
                qs[...] = jnp.dot(_layernorm(xn).astype(BF16), bc(wqu[...]), preferred_element_type=F32)

            NI = 2 * (GH // CH) - 1
            marks = [A1 + DI * i for i in range(NI + 1)] + [NC + A1]

            def start_range(G, lo, hi):
                for k in range(2):
                    a, b = max(lo - k * NC, 0), min(hi - k * NC, NC)
                    if a < b:
                        start_kv(G + 1 + k, a, b)

            def group(G, slot, g, srcs, ahead, extra=None):
                wait_heads(kbuf, slot, g * GH, GH, kv_sem.at[slot, g])
                wait_heads(vbuf, slot, g * GH, GH, kv_sem.at[slot, g])
                for i in range(GH // CH):
                    h0 = g * GH + i * CH
                    pls = [probs(h0 + j, srcs) for j in range(CH)]
                    if extra is not None:
                        extra(i)
                    ahead(2 * i)
                    project(h0, srcs, pls)
                    ahead(2 * i + 1)

            def steady(G, g):
                def ahead(i):
                    if i < NI:
                        start_range(G, marks[i], marks[i + 1])
                    else:
                        start_range(G, marks[i], marks[i] + DI)
                        rest = lambda: start_range(G, marks[i] + DI, marks[i + 1])
                        if isinstance(g, int):
                            if g < NG - 1:
                                rest()
                        else:
                            pl.when(g < NG - 1)(rest)
                return ahead

            def finish_batch(G, active):
                xn = mlp(active)
                start_range(G, marks[NI] + DI, marks[NI] + DI + DM)
                qproj(xn)
                start_range(G, marks[NI] + DI + DM, marks[NI + 1])

            def scatter_rows(dst, t0, h, val):
                if nocomp: return
                r0 = (h // GH) * (GH * DH) + h % GH
                for t in range(val.shape[1] // 128):
                    dst[t0 + t, pl.ds(r0, DH, stride=GH), :] = val[:, 128 * t:128 * t + 128]

            def prep_head_weights(h):
                if nocomp: return
                wt = bc(wqu[:, lanes(h)]).T.astype(F32)
                scatter_rows(qk8, 0, h, wt - jnp.mean(wt, axis=-1, keepdims=True))
                scatter_rows(vo8, TW, h, bc(wou[pl.ds(h * DH // 2, DH // 2), :]).astype(F32))

            def prep_mlp_weights(part, parts):
                if nocomp: return
                blocks = list(range(FM, F, 128))
                for f0 in blocks[part::parts]:
                    n = min(128, F - f0)
                    a = bc(w1u[:, pl.ds(f0, 128)]).T.astype(F32)[:n]
                    a = a - jnp.mean(a, axis=-1, keepdims=True)
                    b = bc(w2u[pl.ds(f0 // 2, n // 2), :]).astype(F32)
                    wm[pl.ds(f0 - FM, n), :] = jnp.concatenate([a, b], axis=1)
                    b1c[pl.ds(f0 - FM, n), :] = jnp.broadcast_to(b1r[0:1, pl.ds(f0, 128)], (128, 128)).T[:n]
                for i in list(range(NX))[part::parts]:
                    a = jnp.concatenate([vo8[TW + t, pl.ds(128 * i, 128), :] for t in range(TD)], axis=1)
                    wox[pl.ds(64 * i, 64), :] = pltpu.bitcast(a.astype(BF16), U32)

            with scope("step0"):
                for g in range(NG):
                    def extra(i, g=g):
                        k = (g * (GH // CH) + i) * HV // (H // CH)
                        for h in range(k, k + HV // (H // CH)):
                            prep_head_weights(h)
                        if g >= NG // 2:
                            prep_mlp_weights((g - NG // 2) * (GH // CH) + i, NG // 2 * (GH // CH))
                    group(g, 0, g, [(0, 0)], steady(g, g), extra)
            with scope("mlpq"):
                finish_batch(NG - 1, row_x == 0)

            def step(s, c):
                slot = s & 1
                def body(g, c):
                    G = s * NG + g
                    group(G, slot, g, [(s - 1, 1 - slot), (s, slot)], steady(G, g))
                    return c
                with scope("grp"):
                    lax.fori_loop(0, NG, body, 0)
                with scope("mlpq"):
                    finish_batch(s * NG + NG - 1, (row_x == s) | (row_x == s - 1))
                return c
            lax.fori_loop(1, last - 1, step, 0)

            s = last - 1
            slot = s % 2
            srcs = [(s - 1, 1 - slot), (s, slot)]

            def keep_kt(g):
                def extra(i):
                    if nocomp: return
                    for j in range(CH):
                        h = g * GH + i * CH + j
                        ktb[h] = pltpu.bitcast(ld(kbuf, slot, h).T, U32)
                return extra

            with scope("grp6"):
                def body(g, c):
                    group(s * NG + g, slot, g, srcs, steady(s * NG + g, g), keep_kt(g))
                    return c
                lax.fori_loop(0, NG - 2, body, 0)
                def ahead(i):
                    if i < NI:
                        start_kv(s * NG + NG - 1, min(marks[i], NC), min(marks[i + 1], NC))
                        start_last(8 * max(marks[i + 1] - NC, 0))
                group(s * NG + NG - 2, slot, NG - 2, srcs, ahead, keep_kt(NG - 2))
                g = NG - 1
                h0 = g * GH
                start_last(T0)
                project(h0, srcs[:1], [probs(h0 + j, srcs[:1]) for j in range(GH)])
                start_last(Q)
            with scope("w63a"):
                wait_heads(kbuf, slot, h0, GH, kv_sem.at[slot, g])
            with scope("w63b"):
                wait_heads(vbuf, slot, h0, GH, kv_sem.at[slot, g])
            with scope("grp63"):
                pls = [probs(h0 + j, srcs[1:]) for j in range(GH)]
                for i in range(GH // CH):
                    keep_kt(g)(i)
                project(h0, srcs[1:], pls)
                start_last(TG[0])
            with scope("mlpq"):
                xn = mlp((row_x == s) | (row_x == s - 1))
                start_last(TG[1])
                qproj(xn)
                start_last(TG[2])

            prev = [(last - 1, 1 - lslot)]
            cur = [(last, lslot)]
            for g in range(NG):
                with scope("kiss%d" % g):
                    start_last((g + 1) * NP + Q)
                with scope("kwait%d" % g):
                    wait_heads(kbuf, lslot, g * GH, GH, k_sem.at[g])
                with scope("kgrp"):
                    h0 = g * GH
                    pls = [probs(h0 + j, prev + cur, prev[0][0]) for j in range(GH)]
                    project(h0, prev, pls)
                    for j, (p, l) in enumerate(pls):
                        if nocomp: break
                        h = h0 + j
                        pbuf[h] = p.astype(F32)
                        lbuf[h] = jnp.broadcast_to(l, (8, DH))
                        kt = ld(kbuf, lslot, h).T
                        if h < HV:
                            scatter_rows(qk8, TD, h, kt.astype(F32))
                        else:
                            ktb[h] = pltpu.bitcast(kt, U32)
                with scope("tg%d" % g):
                    start_last(TG[3 + g])

            done = NG * NP
            for i, (h0, n) in enumerate(v_parts):
                done += n // PAIR * (W // ROWS)
                with scope("viss%d" % i):
                    start_last(done + Q)
                with scope("vwait%d" % i):
                    wait_heads(vbuf, lslot, h0, n, v_sem.at[i])
                with scope("vgrp"):
                    project(h0, cur, [(pbuf[h].astype(BF16), lbuf[h]) for h in range(h0, h0 + n)])
                    for h in range(h0, h0 + n):
                        if h < HV and not nocomp:
                            scatter_rows(vo8, 0, h, ld(vbuf, lslot, h).T.astype(F32))
                if h0 == M6:
                    with scope("mlp6"):
                        start_last(done + 2 * Q)
                        mlp(row_x == last - 1)

            def lanesum(r):
                return jnp.broadcast_to(jnp.sum(r, axis=1, keepdims=True), (8, 128))

            def subsum(a):
                return jnp.broadcast_to(jnp.sum(a, axis=0, keepdims=True), a.shape)

            def total(us):
                r = us[0]
                for u in us[1:]:
                    r = r + u
                return r

            def add_to(accs, t, u):
                accs[t] = u if accs[t] is None else accs[t] + u

            class Paced:
                def __init__(self, vals, lag, every, hist):
                    self.vals, self.lag, self.every, self.hist = list(vals), lag, every, hist

                def get(self):
                    k = len(self.hist)
                    if self.lag and k >= self.lag and k % self.every == 0:
                        z = self.hist[k - self.lag] * 0.0
                        self.vals = [v + z for v in self.vals]
                    return self.vals

            def row_mlp(x1):
                if nocomp: return x1
                d, rs = _center(x1)
                db = d.astype(BF16)
                rsb = jnp.broadcast_to(rs, (8, 128))
                hid, macc, vacc = {}, [None], [None] * TD
                xp = Paced([x1[:, 128 * t:128 * t + 128] for t in range(TD)], LM, PEM, [])

                def up(n0):
                    def f():
                        z = jnp.dot(db, bc(w1u[:, pl.ds(n0, NB)]), preferred_element_type=F32)
                        hid[n0] = _gelu(z * rs + b1r[:, pl.ds(n0, NB)]).astype(BF16)
                    return f

                def down(n0):
                    def f():
                        add_to(macc, 0, jnp.dot(hid[n0], bc(w2u[pl.ds(n0 // 2, NB // 2), :]), preferred_element_type=F32))
                    return f

                def vec(b):
                    def f():
                        xx = xp.get()
                        r = total([wm[pl.ds(8 * b, 8), pl.ds(128 * t, 128)] * xx[t] for t in range(TD)])
                        g = _gelu(lanesum(r) * rsb + b1c[pl.ds(8 * b, 8), :])
                        for t in range(TD):
                            add_to(vacc, t, wm[pl.ds(8 * b, 8), pl.ds(D + 128 * t, 128)] * g)
                        xp.hist.append(vacc[-1])
                    return f

                cost = NB / 128 * 40
                _interleave([(cost, up(n)) for n in range(0, FM, NB)] + [(cost, down(n)) for n in range(0, FM, NB)],
                            [(7, vec(b)) for b in range(FV // 8)])
                return x1 + b2r[...] + macc[0] + subsum(jnp.concatenate(vacc, axis=1))

            def row_attention(x2):
                if nocomp: return x2
                d, rs = _center(x2)
                db = d.astype(BF16)
                sc = rs * scale2
                st, macc, vacc, hist = {}, [None], [None] * TD, []

                def softmax(S):
                    p = jnp.exp2((S - jnp.max(S, axis=1, keepdims=True)) * sc)
                    return p, 1.0 / jnp.sum(p, axis=1, keepdims=True)

                def m_q(h0):
                    def f():
                        st["q", h0] = jnp.dot(db, bc(wqu[:, lanes(h0, MG)]), preferred_element_type=F32).astype(BF16)
                    return f

                def m_qk(h0, j):
                    def f():
                        s = jnp.dot(st["q", h0][:, DH * j:DH * j + DH], bc(ktb[h0 + j]), preferred_element_type=F32)
                        st["S", h0] = s if j == 0 else jnp.where(row_w == j, s, st["S", h0])
                        if j == MG - 1:
                            p, il = softmax(st["S", h0])
                            st["P", h0] = (p.astype(BF16), il)
                    return f

                def m_pv(h0, j):
                    def f():
                        p, il = st["P", h0]
                        o = jnp.dot(p, ld(vbuf, lslot, h0 + j), preferred_element_type=F32)
                        st["A", h0, j] = jnp.where(row_d == j, o * il, 0.0).astype(BF16)
                    return f

                def m_wo(h0):
                    def f():
                        a = jnp.concatenate([st["A", h0, j] for j in range(MG)], axis=1)
                        add_to(macc, 0, jnp.dot(a, bc(wou[pl.ds(h0 * DH // 2, MG * DH // 2), :]), preferred_element_type=F32))
                    return f

                heads = range(HV, H, MG)
                ms = ([(40 * MG, m_q(h0)) for h0 in heads]
                      + [(64, m_qk(h0, j)) for h0 in heads for j in range(MG)]
                      + [(64, m_pv(h0, j)) for h0 in heads for j in range(MG)]
                      + [(40 * MG, m_wo(h0)) for h0 in heads])

                xp = Paced([x2[:, 128 * t:128 * t + 128] for t in range(TD)], L, PE, hist)
                lane = lax.broadcasted_iota(jnp.int32, (8, DH), 1)
                pick = jnp.where((lane & 7) == row_d, lane >> 3, -1)

                def v_qk(g, b):
                    def f():
                        if b == 0:
                            st["vS", g] = [None] * TW
                        rows = pl.ds(g * GH * DH + 8 * b, 8)
                        xx = xp.get()
                        q = lanesum(total([qk8[t, rows, :] * xx[t] for t in range(TD)]))
                        for c in range(TW):
                            add_to(st["vS", g], c, qk8[TD + c, rows, :] * q)
                        hist.append(st["vS", g][-1])
                        if b == DH - 1:
                            p, il = softmax(jnp.concatenate(st["vS", g], axis=1))
                            p = p * il
                            st["vP", g] = [p[:, 128 * c:128 * c + 128] for c in range(TW)]
                    return f

                def v_pv(g, b):
                    def f():
                        if b == 0:
                            st["pp"] = Paced(st["vP", g], L, PE, hist)
                        rows = pl.ds(g * GH * DH + 8 * b, 8)
                        pp = st["pp"].get()
                        o = lanesum(total([vo8[c, rows, :] * pp[c] for c in range(TW)]))
                        if g == 0 and b < 16 * NX:
                            st["X"] = jnp.where(pick == b % 16, o, 0.0 if b % 16 == 0 else st["X"])
                            hist.append(st["X"])
                            if b % 16 == 15:
                                w = bc(wox[pl.ds(64 * (b // 16), 64), :])
                                add_to(macc, 0, jnp.dot(st["X"].astype(BF16), w, preferred_element_type=F32))
                        else:
                            for t in range(TD):
                                add_to(vacc, t, vo8[TW + t, rows, :] * o)
                            hist.append(vacc[-1])
                    return f

                vs = ([(6.5, v_qk(g, b)) for g in range(NV) for b in range(DH)]
                      + [(6.5, v_pv(g, b)) for g in range(NV) for b in range(DH)])
                _interleave(ms, vs)
                return x2 + subsum(macc[0] + jnp.concatenate(vacc, axis=1))

            with scope("mlp1"):
                x = jnp.broadcast_to((xs[...] + acc[...])[last:last + 1], (8, D))
                x = row_mlp(x)
            with scope("attn2"):
                x = row_attention(x)
            with scope("mlp2"):
                x = row_mlp(x)
            with scope("out"):
                out_v[...] = jnp.where(row_x == last, x, xs[...]).astype(out_v.dtype)
                co = pltpu.make_async_copy(out_v, o_hbm, w_sem.at[0])
                co.start()
                co.wait()

        hbm = pl.BlockSpec(memory_space=pltpu.HBM)
        n8 = NV * GH * DH + 8
        out = pl.pallas_call(
            kern,
            out_shape=jax.ShapeDtypeStruct((B, D), A_x.dtype),
            in_specs=[hbm] * 9,
            out_specs=hbm,
            scratch_shapes=[
                pltpu.VMEM((2, H, W, DH), BF16), pltpu.VMEM((2, H, W, DH), BF16),
                pltpu.VMEM((NQ, D // NQ, E), BF16), pltpu.VMEM((NO, E // NO, D), BF16),
                pltpu.VMEM((NW, F // NW, D), BF16), pltpu.VMEM((NW, F // NW, D), BF16),
                pltpu.VMEM((B, D), BF16), pltpu.VMEM((F,), BF16), pltpu.VMEM((D,), BF16),
                pltpu.VMEM((B, D), A_x.dtype),
                pltpu.VMEM((D // 2, E), U32), pltpu.VMEM((E // 2, D), U32),
                pltpu.VMEM((D // 2, FP), U32), pltpu.VMEM((F // 2, D), U32),
                pltpu.VMEM((8, FP), F32), pltpu.VMEM((8, D), F32),
                pltpu.VMEM((B, D), F32), pltpu.VMEM((B, E), F32), pltpu.VMEM((B, D), F32),
                pltpu.VMEM((H, 8, W), F32), pltpu.VMEM((H, 8, DH), F32),
                pltpu.VMEM((H, DH // 2, W), U32),
                pltpu.VMEM((TD + TW, n8, 128), F32), pltpu.VMEM((TD + TW, n8, 128), F32),
                pltpu.VMEM((64 * max(NX, 1), D), U32), pltpu.VMEM((FV, 2 * D), F32), pltpu.VMEM((FV, 128), F32),
                pltpu.SemaphoreType.DMA((2, NG)), pltpu.SemaphoreType.DMA((NG,)),
                pltpu.SemaphoreType.DMA((NG - 1 + len(vparts),)), pltpu.SemaphoreType.DMA((7,)),
            ],
            compiler_params=pltpu.CompilerParams(vmem_limit_bytes=124 * 2**20, disable_bounds_checks=True),
        )(A_x.reshape(B, D), A_k_cache.reshape(B * H, SK, DH), A_v_cache.reshape(B * H, SK, DH),
          A_wq.reshape(NQ, D // NQ, E), A_wo.reshape(NO, E // NO, D), B_w1.T.reshape(NW, F // NW, D), B_b1,
          B_w2.reshape(NW, F // NW, D), B_b2)
        return out.reshape(B, 1, D)
    return run


@jax.jit
def pallas_interleave_layers__sliding_block_cached__mixer_channel_mlp__decode_kernel(A_x, A_k_cache, A_v_cache, A_wq, A_wo, B_x, B_w1, B_b1, B_w2, B_b2):
    return make()(A_x, A_k_cache, A_v_cache, A_wq, A_wo, B_x, B_w1, B_b1, B_w2, B_b2)
```

```python
import jax
import jax.numpy as jnp
from jax import lax
from jax.experimental import pallas as pl
from jax.experimental.pallas import tpu as pltpu

F32, BF16, U32 = jnp.float32, jnp.bfloat16, jnp.uint32
LANES = 128
EPS = 1e-5
LOG2E = 1.4426950408889634

GROUP, PAIR, ROWS = 8, 2, 64
AHEAD, STEP, MID = 14, 2, 3
LEAD = 116
LAST_MARKS = (40, 152, 176, 204, 253, 301, 344, 387)

TAIL = dict(
    mxu_ff=1280,
    ff_block=256,
    mxu_heads=8,
    moved=(4, 1),
    pace_keys=((16, 4), (16, 4)),
    pace_values=((20, 4), (20, 5)),
    pace_moved=(32, 8),
    warmup=(32, 0.25),
    overlap=96,
    weight_attention=1.2,
    weight_mlp=0.8,
)


def _bf16(words):
    return pltpu.bitcast(words, BF16)


def _matmul(a, b):
    return jnp.dot(a, b, preferred_element_type=F32)


def _layernorm(x):
    d = x - jnp.mean(x, axis=-1, keepdims=True)
    return d * lax.rsqrt(jnp.mean(d * d, axis=-1, keepdims=True) + EPS)


def _stats(x):
    m = jnp.mean(x, axis=-1, keepdims=True)
    d = x - m
    return m, lax.rsqrt(jnp.mean(d * d, axis=-1, keepdims=True) + EPS)


def _gelu(x):
    c = 0.7978845608028654
    return (0.5 * x) * (1.0 + jnp.tanh(x * (c + (c * 0.044715) * (x * x))))


def _loop(lo, hi, fn):
    if hi > lo:
        lax.fori_loop(lo, hi, lambda i, carry: (fn(i), carry)[1], 0)


def _times(i, n):
    return i * n if isinstance(i, int) else pl.multiple_of(i * n, n)


def _tiles(x):
    return [x[:, LANES * t:LANES * (t + 1)] for t in range(x.shape[1] // LANES)]


def _sum(terms):
    total = terms[0]
    for term in terms[1:]:
        total = total + term
    return total


def _lane_sum(x):
    return jnp.broadcast_to(jnp.sum(x, axis=1, keepdims=True), x.shape)


def _row_sum(x):
    return jnp.broadcast_to(jnp.sum(x, axis=0, keepdims=True), x.shape)


def _accumulate(totals, i, term):
    totals[i] = term if totals[i] is None else totals[i] + term


def _interleave(*streams):
    pos, spent = [0] * len(streams), [0.0] * len(streams)
    while True:
        live = [i for i in range(len(streams)) if pos[i] < len(streams[i])]
        if not live:
            return
        i = min(live, key=lambda i: spent[i])
        cost, thunk = streams[i][pos[i]]
        thunk()
        pos[i] += 1
        spent[i] += cost


class _Paced:
    def __init__(self, values, results):
        self.values, self.results, self.uses = list(values), results, 0

    def get(self, lag, period, first_lag=0, decay=0.0):
        lag = max(lag, int(first_lag - max(self.uses - first_lag, 0) * decay))
        if len(self.results) >= lag and self.uses % period == 0:
            zero = self.results[len(self.results) - lag] * 0.0
            self.values = [v + zero for v in self.values]
        self.uses += 1
        return self.values


def _row_mlp(cfg, x, w1, w2, b1, b2, w1_sum, vec_w, vec_b1):
    d = x.shape[1]
    block = cfg["ff_block"]
    mean, scale = _stats(x)
    lhs = x.astype(BF16)
    scale_tile = jnp.broadcast_to(scale, (8, LANES))
    x_tiles = _tiles(x)
    hidden, mxu_out, vec_out = {}, [None], [None] * (d // LANES)

    def up(f):
        cols = pl.ds(f, block)
        z = _matmul(lhs, _bf16(w1[:, cols])) - mean * w1_sum[:, cols]
        hidden[f] = _gelu(z * scale + b1[:, cols]).astype(BF16)

    def down(f):
        _accumulate(mxu_out, 0, _matmul(hidden[f], _bf16(w2[pl.ds(f // 2, block // 2), :])))

    def vector(i):
        rows = pl.ds(8 * i, 8)
        z = _lane_sum(_sum([vec_w[rows, pl.ds(LANES * t, LANES)] * xt for t, xt in enumerate(x_tiles)]))
        h = _gelu(z * scale_tile + vec_b1[rows, :])
        for t in range(len(vec_out)):
            _accumulate(vec_out, t, vec_w[rows, pl.ds(d + LANES * t, LANES)] * h)

    cost = block / LANES * 40
    starts = range(0, cfg["mxu_ff"], block)
    _interleave([(cost, lambda f=f: up(f)) for f in starts] + [(cost, lambda f=f: down(f)) for f in starts],
                [(7 * cfg["weight_mlp"], lambda i=i: vector(i)) for i in range(vec_w.shape[0] // 8)])
    return x + b2[...] + mxu_out[0] + _row_sum(jnp.concatenate(vec_out, axis=1))


def _row_attention(cfg, x, exp_scale, wq, wq_sum, wo, keys_t, load_values, vec_qk, vec_vo, moved_wo, vec_heads, heads):
    n_x, dh = x.shape[1] // LANES, LANES
    n_w = vec_qk.shape[0] - n_x
    block = cfg["mxu_heads"]
    mean, scale = _stats(x)
    lhs = x.astype(BF16)
    scale = scale * exp_scale
    state, mxu_out, vec_out, results = {}, [None], [None] * n_x, []
    row_w = lax.broadcasted_iota(jnp.int32, (8, n_w * LANES), 0)
    row_d = lax.broadcasted_iota(jnp.int32, (8, dh), 0)
    lane = lax.broadcasted_iota(jnp.int32, (8, dh), 1)

    def softmax(s):
        p = jnp.exp2((s - jnp.max(s, axis=1, keepdims=True)) * scale)
        return p, 1.0 / jnp.sum(p, axis=1, keepdims=True)

    def mxu_query(h0):
        cols = pl.ds(h0 * dh, block * dh)
        state["q", h0] = (_matmul(lhs, _bf16(wq[:, cols])) - mean * wq_sum[:, cols]).astype(BF16)

    def mxu_keys(h0, j):
        s = _matmul(state["q", h0][:, dh * j:dh * (j + 1)], _bf16(keys_t[h0 + j]))
        state["s", h0] = s if j == 0 else jnp.where(row_w == j, s, state["s", h0])
        if j == block - 1:
            p, norm = softmax(state["s", h0])
            state["p", h0] = (p.astype(BF16), norm)

    def mxu_values(h0, j):
        p, norm = state["p", h0]
        state["o", h0, j] = jnp.where(row_d == j, _matmul(p, load_values(h0 + j)) * norm, 0.0).astype(BF16)

    def mxu_output(h0):
        o = jnp.concatenate([state["o", h0, j] for j in range(block)], axis=1)
        _accumulate(mxu_out, 0, _matmul(o, _bf16(wo[pl.ds(h0 * dh // 2, block * dh // 2), :])))

    stages = (lambda h0: [(40 * block, lambda: mxu_query(h0))],
              lambda h0: [(64, lambda j=j: mxu_keys(h0, j)) for j in range(block)],
              lambda h0: [(64, lambda j=j: mxu_values(h0, j)) for j in range(block)],
              lambda h0: [(40 * block, lambda: mxu_output(h0))])
    starts = list(range(vec_heads, heads, block))
    mxu_work = []
    for i in range(len(starts) + len(stages) - 1):
        for lag, stage in enumerate(stages):
            if 0 <= i - lag < len(starts):
                mxu_work += stage(starts[i - lag])

    paced_x = _Paced(_tiles(x), results)
    slot = jnp.where((lane & (GROUP - 1)) == row_d, lane >> 3, -1)

    def vec_keys(g, i):
        if i == 0:
            state["vs", g] = [None] * n_w
        rows = pl.ds(g * GROUP * dh + GROUP * i, GROUP)
        xs = paced_x.get(*cfg["pace_keys"][g], *(() if g else cfg["warmup"]))
        q = _lane_sum(_sum([vec_qk[t, rows, :] * xs[t] for t in range(n_x)]))
        for t in range(n_w):
            _accumulate(state["vs", g], t, vec_qk[n_x + t, rows, :] * q)
        results.append(state["vs", g][0])
        if i == dh - 1:
            p, norm = softmax(jnp.concatenate(state["vs", g], axis=1))
            state["vp", g] = _Paced(_tiles(p * norm), results)

    def vec_values(g, i):
        rows = pl.ds(g * GROUP * dh + GROUP * i, GROUP)
        moved = i < 16 * cfg["moved"][g]
        ps = state["vp", g].get(*(cfg["pace_moved"] if moved else cfg["pace_values"][g]))
        o = _lane_sum(_sum([vec_vo[t, rows, :] * ps[t] for t in range(n_w)]))
        if moved:
            state["lhs"] = jnp.where(slot == i % 16, o, 0.0 if i % 16 == 0 else state["lhs"])
            results.append(state["lhs"])
            if i % 16 == 15:
                w = moved_wo[pl.ds(64 * (g * cfg["moved"][0] + i // 16), 64), :]
                _accumulate(mxu_out, 0, _matmul(state["lhs"].astype(BF16), _bf16(w)))
        else:
            for t in range(n_x):
                _accumulate(vec_out, t, vec_vo[n_w + t, rows, :] * o)
            results.append(vec_out[0])

    cost, k = 6.5 * cfg["weight_attention"], cfg["overlap"]
    spans = ((vec_keys, 0, 0, dh), (vec_keys, 1, 0, k), (vec_values, 0, 0, dh - k),
             (vec_keys, 1, k, dh), (vec_values, 0, dh - k, dh), (vec_values, 1, 0, dh))
    _interleave(mxu_work, [(cost, lambda fn=fn, g=g, i=i: fn(g, i)) for fn, g, lo, hi in spans for i in range(lo, hi)])
    return x + _row_sum(mxu_out[0] + jnp.concatenate(vec_out, axis=1))


def _make_kernel(cfg, batch, heads, seq, window):
    dh = LANES
    n_groups, n_chunks, half = heads // GROUP, window // ROWS, GROUP // 2
    vec_heads = 2 * GROUP
    last = batch - 1
    last_slot = last % 2
    exp_scale = dh ** -0.5 * LOG2E

    def kernel(x_hbm, k_hbm, v_hbm, wq_hbm, wo_hbm, w1t_hbm, b1_hbm, w2_hbm, b2_hbm, o_hbm,
               kbuf, vbuf, wq_in, wo_in, w1t_in, w2_in, x_in, b1_in, b2_in, out,
               wq, wo, w1, w2, wq_sum, w1_sum, b1, b2, xs, qs, acc, p_last, l_last,
               keys_t, vec_qk, vec_vo, moved_wo, vec_w, vec_b1,
               kv_sem, last_sem, w_sem):
        d, ff = xs.shape[1], b1_in.shape[0]
        n_x, n_w = d // LANES, window // LANES

        def load(buf, *idx):
            return _bf16(buf.bitcast(U32)[idx])

        def kv_copy(src, dst, src_head, slot, head, row, sem):
            return pltpu.make_async_copy(src.at[pl.ds(src_head, PAIR), pl.ds(seq - window + row, ROWS), :],
                                         dst.at[slot, pl.ds(head, PAIR), pl.ds(row, ROWS), :], sem)

        def start_group(n, lo, hi):
            if isinstance(n, int):
                slot, g = (n // n_groups) % 2, n % n_groups
            else:
                slot, g = lax.shift_right_logical(n, n_groups.bit_length() - 1) & 1, n & (n_groups - 1)

            def chunk(i):
                row = _times(i, ROWS)
                for h in range(0, GROUP, PAIR):
                    kv_copy(k_hbm, kbuf, n * GROUP + h, slot, g * GROUP + h, row, kv_sem.at[0, slot, g]).start(priority=0)
                    kv_copy(v_hbm, vbuf, n * GROUP + h, slot, g * GROUP + h, row, kv_sem.at[1, slot, g]).start(priority=1)
            _loop(lo, hi, chunk)

        def start_after(n, lo, hi):
            for k in range(2):
                start_group(n + 1 + k, max(lo - k * n_chunks, 0), min(hi - k * n_chunks, n_chunks))

        def wait(region, sem):
            pltpu.make_async_copy(region, region, sem).wait()

        def wait_group(slot, g):
            wait(kbuf.at[slot, pl.ds(g * GROUP, GROUP)], kv_sem.at[0, slot, g])
            wait(vbuf.at[slot, pl.ds(g * GROUP, GROUP)], kv_sem.at[1, slot, g])

        parts = [(src, dst, g * GROUP) for src, dst in ((k_hbm, kbuf), (v_hbm, vbuf)) for g in range(n_groups)]
        per_chunk = GROUP // PAIR
        per_part = n_chunks * per_chunk
        end_rows = window // 4
        pieces = [(heads - 2 * GROUP, half, 0, window), (heads - GROUP - half, half, 0, window),
                  (heads - GROUP, half, 0, window), (heads - half, PAIR, 0, window),
                  (heads - PAIR, PAIR, 0, window - end_rows), (heads - PAIR, PAIR, window - end_rows, end_rows)]
        started = [0]

        def piece_sem(n):
            return last_sem.at[len(parts) - 2 + n]

        def start_last(upto):
            for i, (src, dst, h0) in enumerate(parts):
                lo, hi = (min(max((e - i * per_part) // per_chunk, 0), n_chunks) for e in (started[0], upto))
                whole = i < len(parts) - 2
                sem0 = last_sem.at[i] if whole else piece_sem(2 * (i - len(parts) + 2))
                sem1 = last_sem.at[i] if whole else piece_sem(1)

                def chunk(k, late=None, src=src, dst=dst, h0=h0, sem0=sem0, sem1=sem1):
                    for j, h in enumerate(range(h0, h0 + half, PAIR)):
                        kv_copy(src, dst, last * heads + h, last_slot, h, _times(k, ROWS), sem0).start(priority=0)
                        if late is None:
                            h1, c, sem = h + half, k, sem1
                        else:
                            h1, c, sem = late[0], 2 * (k - late[1]) + j, late[2]
                        kv_copy(src, dst, last * heads + h1, last_slot, h1, _times(c, ROWS), sem).start(priority=1)

                if i < len(parts) - 1:
                    _loop(lo, hi, chunk)
                    continue
                for n, (h1, _, r0, nr) in list(enumerate(pieces))[3:]:
                    k0 = (h1 - (heads - half)) // PAIR * (n_chunks // 2)
                    a, b = k0 + r0 // (2 * ROWS), k0 + (r0 + nr) // (2 * ROWS)
                    _loop(max(lo, a), min(hi, b), lambda k, late=(h1, k0, piece_sem(n)): chunk(k, late))
            started[0] = max(started[0], upto)

        def receive_last(i):
            _, dst, h0 = parts[i]
            start_last((i + 1) * per_part + LEAD)
            wait(dst.at[last_slot, pl.ds(h0, GROUP)], last_sem.at[i])

        def start_weights(src0, dst0, sem0, cols, src1, dst1, sem1):
            n0, ratio = src0.shape[1] // 8, src1.shape[1] // src0.shape[1]

            def strip(i):
                rows0 = pl.ds(_times(i, 8), 8)
                for k in range(ratio):
                    cols0, rows1 = pl.ds(k * cols, cols), pl.ds(_times(i * ratio + k, 8), 8)
                    pltpu.make_async_copy(src0.at[:, rows0, cols0], dst0.at[:, rows0, cols0], sem0).start(priority=0)
                    pltpu.make_async_copy(src1.at[:, rows1], dst1.at[:, rows1], sem1).start(priority=1)
            _loop(0, n0, strip)

        def repack(src, dst):
            n = src.shape[1] // 2

            def part(i):
                dst[pl.ds(_times(i, n), n), :] = pltpu.bitcast(src[i], U32)
            _loop(0, src.shape[0], part)

        row_w = lax.broadcasted_iota(jnp.int32, (8, window), 0)
        row_d = lax.broadcasted_iota(jnp.int32, (8, dh), 0)
        row_x = lax.broadcasted_iota(jnp.int32, (8, d), 0)

        small = [pltpu.make_async_copy(src, dst, w_sem.at[i])
                 for i, (src, dst) in enumerate(((x_hbm, x_in), (b1_hbm, b1_in), (b2_hbm, b2_in)))]
        for copy in small:
            copy.start()
        start_weights(wq_hbm, wq_in, w_sem.at[3], 512, wo_hbm, wo_in, w_sem.at[4])
        start_weights(w1t_hbm, w1t_in, w_sem.at[5], d, w2_hbm, w2_in, w_sem.at[6])

        small[0].wait()
        x0 = x_in[...].astype(F32)
        xs[...] = x0
        acc[...] = jnp.zeros_like(acc)
        wait(wq_in, w_sem.at[3])
        repack(wq_in, wq)
        start_group(0, 0, n_chunks // 2)
        q0 = _matmul(jnp.concatenate([_layernorm(x0), jnp.ones((8, d), F32)], axis=0).astype(BF16), _bf16(wq[...]))
        qs[...] = q0[:8]
        wq_sum[...] = q0[8:]
        start_group(0, n_chunks // 2, n_chunks)
        wait(wo_in, w_sem.at[4])
        repack(wo_in, wo)
        start_group(1, 0, AHEAD // 2)
        small[1].wait()
        small[2].wait()
        wait(w1t_in, w_sem.at[5])
        wait(w2_in, w_sem.at[6])
        repack(w2_in, w2)
        w1t = w1t_in[...].reshape(ff, d)
        for f in range(0, ff, LANES):
            rows = w1t[f:f + LANES]
            if rows.shape[0] < LANES:
                rows = jnp.concatenate([rows, jnp.zeros((LANES - rows.shape[0], d), BF16)], axis=0)
            w1[:, pl.ds(f, LANES)] = pltpu.bitcast(rows.T, U32)
        w1_sum[...] = _matmul(jnp.ones((8, d), BF16), _bf16(w1[...]))
        bias = b1_in[...].astype(F32).reshape(1, ff)
        bias = jnp.concatenate([bias, jnp.zeros((1, b1.shape[1] - ff), F32)], axis=1)
        b1[...] = jnp.broadcast_to(bias, b1.shape)
        b2[...] = jnp.broadcast_to(b2_in[...].astype(F32).reshape(1, d), b2.shape)
        start_group(1, AHEAD // 2, AHEAD)

        def probs(h, prev, cur):
            q = qs[:, pl.ds(_times(h, dh), dh)].astype(BF16)
            s = None
            if prev is not None:
                s = _matmul(q, _bf16(keys_t[h]))
            if cur is not None:
                fresh = lax.dot_general(q, load(kbuf, cur[1], h), (((1,), (1,)), ((), ())), preferred_element_type=F32)
                s = fresh if s is None else jnp.where(row_w == cur[0], fresh, s)
            p = jnp.exp2((s - jnp.max(s, axis=-1, keepdims=True)) * exp_scale)
            return p.astype(BF16), jnp.sum(p, axis=-1, keepdims=True)

        def keep_keys(h, slot):
            keys_t[h] = pltpu.bitcast(load(kbuf, slot, h).T, U32)

        def project(h0, rows, weights):
            outs = []
            for j, (p, total) in enumerate(weights):
                o, norm = jnp.zeros((8, dh), F32), 1.0 / total
                for row, slot in rows:
                    o = jnp.where(row_d == row, _matmul(p, load(vbuf, slot, h0 + j)) * norm, o)
                outs.append(o.astype(BF16))
            w = wo[pl.ds(_times(h0, dh // 2), len(weights) * dh // 2), :]
            acc[...] += _matmul(jnp.concatenate(outs, axis=-1), _bf16(w))

        def mlp(active):
            x1 = xs[...] + acc[...]
            h = _gelu(_matmul(_layernorm(x1).astype(BF16), _bf16(w1[...])) + b1[...])[:, :ff]
            x2 = jnp.where(active, x1 + _matmul(h.astype(BF16), _bf16(w2[...])) + b2[...], xs[...])
            xs[...] = x2
            acc[...] = jnp.where(active, 0.0, acc[...])
            return x2

        def queries(x):
            qs[...] = _matmul(_layernorm(x).astype(BF16), _bf16(wq[...]))

        marks = [AHEAD + STEP * i for i in range(5)]

        def group(b, g, prev, start, extra=None):
            slot = b & 1
            wait_group(slot, g)
            rows = ([] if prev is None else [(prev, 1 - slot)]) + [(b, slot)]
            for i in range(2):
                h0 = g * GROUP + i * half
                weights = [probs(h0 + j, prev, (b, slot)) for j in range(half)]
                for j in range(half):
                    keep_keys(h0 + j, slot)
                start(2 * i)
                project(h0, rows, weights)
                if extra is not None:
                    extra(i)
                start(2 * i + 1)

        def whole_batch(b, prev, extra):
            def body(g):
                n = b * n_groups + g
                group(b, g, prev, lambda i: start_after(n, marks[i], marks[i + 1]), lambda i: extra(2 * g + i))
                pl.when(g < n_groups - 1)(lambda: start_after(n, marks[-1], n_chunks + AHEAD))
            _loop(0, n_groups, body)
            n = b * n_groups + n_groups - 1
            x = mlp(row_x == b if prev is None else (row_x == b) | (row_x == prev))
            start_after(n, marks[-1], marks[-1] + MID)
            queries(x)
            start_after(n, marks[-1] + MID, n_chunks + AHEAD)

        def spread(dst, first_tile, h, value):
            g, j = divmod(h, GROUP) if isinstance(h, int) else (lax.shift_right_logical(h, 3), h & (GROUP - 1))
            for t, tile in enumerate(_tiles(value)):
                dst[first_tile + t, pl.ds(g * (GROUP * dh) + j, dh, stride=GROUP), :] = tile

        def prepare_heads(k):
            n = vec_heads * half // heads
            for j in range(n):
                h = k * n + j
                cols = _bf16(wq[:, pl.ds(_times(h, dh), dh)]).T.astype(F32)
                spread(vec_qk, 0, h, cols - jnp.mean(cols, axis=-1, keepdims=True))
                spread(vec_vo, n_w, h, _bf16(wo[pl.ds(_times(h, dh // 2), dh // 2), :]).astype(F32))

        def prepare_hidden(k, n):
            f = _times(cfg["mxu_ff"] // LANES + k, LANES)
            up = _bf16(w1[:, pl.ds(f, LANES)]).T.astype(F32)[:n]
            down = _bf16(w2[pl.ds(_times(cfg["mxu_ff"] // LANES + k, LANES // 2), n // 2), :]).astype(F32)
            rows = pl.ds(_times(k, LANES), n)
            vec_w[rows, :] = jnp.concatenate([up - jnp.mean(up, axis=-1, keepdims=True), down], axis=1)
            vec_b1[rows, :] = jnp.broadcast_to(b1[0:1, pl.ds(f, LANES)], (LANES, LANES)).T[:n]

        def prepare_moved(i):
            r = jnp.where(i < cfg["moved"][0], i, i - cfg["moved"][0] + GROUP)
            rows = [vec_vo[n_w + t, pl.ds(_times(r, LANES), LANES), :] for t in range(n_x)]
            moved_wo[pl.ds(_times(i, 64), 64), :] = pltpu.bitcast(jnp.concatenate(rows, axis=1).astype(BF16), U32)

        whole_batch(0, None, prepare_heads)

        def step(b):
            def extra(k):
                full, rest = divmod(vec_w.shape[0], LANES)

                @pl.when(b == 1)
                def _():
                    pl.when(k < full)(lambda: prepare_hidden(k, LANES))
                    if rest:
                        pl.when(k == full)(lambda: prepare_hidden(full, rest))
                i = (b - 2) * (2 * n_groups) + k
                pl.when((b >= 2) & (i < sum(cfg["moved"])))(lambda: prepare_moved(i))
            whole_batch(b, b - 1, extra)
        _loop(1, last - 1, step)

        b = last - 1
        slot = b % 2

        def body(g):
            n = b * n_groups + g
            group(b, g, b - 1, lambda i: start_after(n, marks[i], marks[i + 1] if i < 3 else n_chunks + AHEAD))
        _loop(0, n_groups - 2, body)

        def start(i):
            start_group(last * n_groups - 1, min(marks[i], n_chunks), min(marks[i + 1], n_chunks))
            start_last(2 * per_chunk * max(marks[i + 1] - n_chunks, 0))
        group(b, n_groups - 2, b - 1, start)

        h0 = heads - GROUP
        start_last(LAST_MARKS[0])
        project(h0, [(b - 1, 1 - slot)], [probs(h0 + j, b - 1, None) for j in range(GROUP)])
        start_last(LEAD)
        wait_group(slot, n_groups - 1)
        weights = [probs(h0 + j, None, (b, slot)) for j in range(GROUP)]
        for j in range(GROUP):
            keep_keys(h0 + j, slot)
        project(h0, [(b, slot)], weights)
        start_last(LAST_MARKS[1])
        x = mlp((row_x == b) | (row_x == b - 1))
        start_last(LAST_MARKS[2])
        queries(x)
        start_last(LAST_MARKS[3])

        for g in range(n_groups):
            receive_last(g)
            h0 = g * GROUP
            weights = [probs(h0 + j, last - 1, (last, last_slot)) for j in range(GROUP)]
            project(h0, [(last - 1, 1 - last_slot)], weights)
            for h, (p, total) in enumerate(weights, h0):
                p_last[h] = jnp.broadcast_to(p.astype(F32)[last:last + 1], (8, window))
                l_last[h] = jnp.broadcast_to(total[last:last + 1], (8, dh))
                if h < vec_heads:
                    spread(vec_qk, n_x, h, load(kbuf, last_slot, h).T.astype(F32))
                else:
                    keep_keys(h, last_slot)
            start_last(LAST_MARKS[4 + g])
        mlp(row_x == last - 1)
        for g in range(vec_heads // GROUP):
            receive_last(n_groups + g)
            hs = range(g * GROUP, (g + 1) * GROUP)
            project(g * GROUP, [(last, last_slot)], [(p_last[h].astype(BF16), l_last[h]) for h in hs])
            for h in hs:
                spread(vec_vo, 0, h, load(vbuf, last_slot, h).T.astype(F32))
        start_last(len(parts) * per_part)

        partial = {}
        x = jnp.broadcast_to((xs[...] + acc[...])[last:last + 1], (8, d))
        for n, (h0, nh, r0, nr) in enumerate(pieces):
            wait(vbuf.at[last_slot, pl.ds(h0, nh), pl.ds(r0, nr)], piece_sem(n))
            for h in range(h0, h0 + nh):
                o = _matmul(p_last[h, :, pl.ds(r0, nr)].astype(BF16), load(vbuf, last_slot, h, pl.ds(r0 // 2, nr // 2)))
                partial[h] = o + partial[h] if r0 else o
            if r0 + nr == window:
                o = jnp.concatenate([partial[h] * (1.0 / l_last[h]) for h in range(h0, h0 + nh)], axis=-1).astype(BF16)
                x = x + _matmul(o, _bf16(wo[pl.ds(h0 * dh // 2, nh * dh // 2), :]))

        x = _row_mlp(cfg, x, w1, w2, b1, b2, w1_sum, vec_w, vec_b1)
        x = _row_attention(cfg, x, exp_scale, wq, wq_sum, wo, keys_t, lambda h: load(vbuf, last_slot, h),
                           vec_qk, vec_vo, moved_wo, vec_heads, heads)
        x = _row_mlp(cfg, x, w1, w2, b1, b2, w1_sum, vec_w, vec_b1)
        out[...] = jnp.where(row_x == last, x, xs[...]).astype(out.dtype)
        copy = pltpu.make_async_copy(out, o_hbm, w_sem.at[0])
        copy.start()
        copy.wait()

    return kernel


def _run(cfg, x, k_cache, v_cache, wq, wo, w1, b1, w2, b2):
    batch, _, d = x.shape
    _, heads, seq, dh = k_cache.shape
    window = min(4096, max(256, seq // 4))
    ff, e = w1.shape[1], heads * dh
    ff_padded = pl.cdiv(ff, LANES) * LANES
    assert (batch, heads, dh) == (8, 4 * GROUP, LANES) and d % LANES == 0
    wq, wo = wq.reshape(5, d // 5, e), wo.reshape(4, e // 4, d)
    w1t, w2 = w1.T.reshape(4, ff // 4, d), w2.reshape(4, ff // 4, d)
    vec_ff = ff - cfg["mxu_ff"]
    vec_rows = 2 * GROUP * dh + 8

    vmem, dma, hbm = pltpu.VMEM, pltpu.SemaphoreType.DMA, pl.BlockSpec(memory_space=pltpu.HBM)
    out = pl.pallas_call(
        _make_kernel(cfg, batch, heads, seq, window),
        out_shape=jax.ShapeDtypeStruct((batch, d), x.dtype),
        in_specs=[hbm] * 9,
        out_specs=hbm,
        scratch_shapes=[
            vmem((2, heads, window, dh), BF16), vmem((2, heads, window, dh), BF16),
            vmem(wq.shape, BF16), vmem(wo.shape, BF16), vmem(w1t.shape, BF16), vmem(w2.shape, BF16),
            vmem((batch, d), BF16), vmem((ff,), BF16), vmem((d,), BF16), vmem((batch, d), x.dtype),
            vmem((d // 2, e), U32), vmem((e // 2, d), U32), vmem((d // 2, ff_padded), U32), vmem((ff // 2, d), U32),
            vmem((8, e), F32), vmem((8, ff_padded), F32), vmem((8, ff_padded), F32), vmem((8, d), F32),
            vmem((batch, d), F32), vmem((batch, e), F32), vmem((batch, d), F32),
            vmem((heads, 8, window), F32), vmem((heads, 8, dh), F32),
            vmem((heads, dh // 2, window), U32),
            vmem(((d + window) // LANES, vec_rows, LANES), F32), vmem(((d + window) // LANES, vec_rows, LANES), F32),
            vmem((64 * sum(cfg["moved"]), d), U32), vmem((vec_ff, 2 * d), F32), vmem((vec_ff, LANES), F32),
            dma((2, 2, heads // GROUP)), dma((2 * heads // GROUP + 4,)), dma((7,)),
        ],
        compiler_params=pltpu.CompilerParams(vmem_limit_bytes=124 * 2**20, disable_bounds_checks=True),
    )(x.reshape(batch, d), k_cache.reshape(batch * heads, seq, dh), v_cache.reshape(batch * heads, seq, dh),
      wq, wo, w1t, b1, w2, b2)
    return out.reshape(batch, 1, d)


@jax.jit
def pallas_interleave_layers__sliding_block_cached__mixer_channel_mlp__decode_kernel(
    A_x: jax.Array,
    A_k_cache: jax.Array,
    A_v_cache: jax.Array,
    A_wq: jax.Array,
    A_wo: jax.Array,
    B_x: jax.Array,
    B_w1: jax.Array,
    B_b1: jax.Array,
    B_w2: jax.Array,
    B_b2: jax.Array,
):
    del B_x
    return _run(TAIL, A_x, A_k_cache, A_v_cache, A_wq, A_wo, B_w1, B_b1, B_w2, B_b2)
```

```python
import jax
import jax.numpy as jnp
from jax import lax
from jax.experimental import pallas as pl
from jax.experimental.pallas import tpu as pltpu

F32, BF16, U32 = jnp.float32, jnp.bfloat16, jnp.uint32
LANES = 128
EPS = 1e-5
LOG2E = 1.4426950408889634

GROUP, PAIR, ROWS = 8, 2, 64
AHEAD, STEP, MID = 15, 3, 3
LEAD = 116
LAST_MARKS = (152, 176, 204, 253, 301, 344, 387)

MXU_FF = 1152
MOVED = 4
PACE_MLP, PACE_KEYS, PACE_MOVED, PACE_VALUES = (24, 4), (16, 4, 40), (36, 6), ((20, 5), (24, 8))


def _bf16(words):
    return pltpu.bitcast(words, BF16)


def _matmul(a, b):
    return jnp.dot(a, b, preferred_element_type=F32)


def _layernorm(x):
    d = x - jnp.mean(x, axis=-1, keepdims=True)
    return d * lax.rsqrt(jnp.mean(d * d, axis=-1, keepdims=True) + EPS)


def _stats(x):
    m = jnp.mean(x, axis=-1, keepdims=True)
    d = x - m
    return m, lax.rsqrt(jnp.mean(d * d, axis=-1, keepdims=True) + EPS)


def _gelu(x):
    c = 0.7978845608028654
    return (0.5 * x) * (1.0 + jnp.tanh(x * (c + (c * 0.044715) * (x * x))))


def _loop(lo, hi, fn):
    if hi > lo:
        lax.fori_loop(lo, hi, lambda i, carry: (fn(i), carry)[1], 0)


def _times(i, n):
    return i * n if isinstance(i, int) else pl.multiple_of(i * n, n)


def _tiles(x):
    return [x[:, LANES * t:LANES * (t + 1)] for t in range(x.shape[1] // LANES)]


def _sum(terms, pairwise=False):
    while pairwise and len(terms) > 1:
        terms = [terms[i] + terms[i + 1] if i + 1 < len(terms) else terms[i] for i in range(0, len(terms), 2)]
    total = terms[0]
    for term in terms[1:]:
        total = total + term
    return total


def _lane_sum(x):
    return jnp.broadcast_to(jnp.sum(x, axis=1, keepdims=True), x.shape)


def _row_sum(x):
    return jnp.broadcast_to(jnp.sum(x, axis=0, keepdims=True), x.shape)


def _accumulate(totals, i, term):
    totals[i] = term if totals[i] is None else totals[i] + term


def _interleave(*streams):
    pos, spent = [0] * len(streams), [0.0] * len(streams)
    while True:
        live = [i for i in range(len(streams)) if pos[i] < len(streams[i])]
        if not live:
            return
        i = min(live, key=lambda i: spent[i])
        cost, thunk = streams[i][pos[i]]
        thunk()
        pos[i] += 1
        spent[i] += cost


class _Paced:
    def __init__(self, values, results):
        self.values, self.results, self.uses = list(values), results, 0

    def get(self, lag, period, first_lag=0):
        lag = max(lag, first_lag - max(self.uses - first_lag, 0))
        if len(self.results) >= lag and self.uses % period == 0:
            zero = self.results[len(self.results) - lag] * 0.0
            self.values = [v + zero for v in self.values]
        self.uses += 1
        return self.values


def _row_mlp(x, w1, w2, b1, b2, w1_sum, vec_w, vec_b1):
    d = x.shape[1]
    mean, scale = _stats(x)
    lhs = x.astype(BF16)
    paced_scale = _Paced([jnp.broadcast_to(scale, (8, LANES))], [])
    x_tiles = _tiles(x)
    hidden, mxu_out, vec_out = {}, [None], [None] * (d // LANES)

    def up(f):
        cols = pl.ds(f, LANES)
        z = _matmul(lhs, _bf16(w1[:, cols])) - mean * w1_sum[:, cols]
        hidden[f] = _gelu(z * scale + b1[:, cols]).astype(BF16)

    def down(f):
        _accumulate(mxu_out, 0, _matmul(hidden[f], _bf16(w2[pl.ds(f // 2, LANES // 2), :])))

    def vector(i):
        rows = pl.ds(8 * i, 8)
        z = _lane_sum(_sum([vec_w[rows, pl.ds(LANES * t, LANES)] * xt for t, xt in enumerate(x_tiles)]))
        h = _gelu(z * paced_scale.get(*PACE_MLP)[0] + vec_b1[rows, :])
        for t in range(len(vec_out)):
            _accumulate(vec_out, t, vec_w[rows, pl.ds(d + LANES * t, LANES)] * h)
        paced_scale.results.append(vec_out[0])

    starts = range(0, MXU_FF, LANES)
    _interleave([(40, lambda f=f: up(f)) for f in starts] + [(40, lambda f=f: down(f)) for f in starts],
                [(3.5, lambda i=i: vector(i)) for i in range(vec_w.shape[0] // 8)])
    return x + b2[...] + mxu_out[0] + _row_sum(jnp.concatenate(vec_out, axis=1))


def _row_attention(x, exp_scale, wq, wq_sum, wo, keys_t, values, vec_qk, vec_vo, moved_wo, vec_heads, heads):
    n_x, dh = x.shape[1] // LANES, LANES
    n_w = vec_qk.shape[0] - n_x
    mean, scale = _stats(x)
    lhs = x.astype(BF16)
    scale = scale * exp_scale
    state, mxu_out, vec_out, results = {}, [None], [None] * n_x, []
    row_w = lax.broadcasted_iota(jnp.int32, (8, n_w * LANES), 0)
    row_d = lax.broadcasted_iota(jnp.int32, (8, dh), 0)
    lane = lax.broadcasted_iota(jnp.int32, (8, dh), 1)

    def softmax(s):
        p = jnp.exp2((s - jnp.max(s, axis=1, keepdims=True)) * scale)
        return p, 1.0 / jnp.sum(p, axis=1, keepdims=True)

    def mxu_query(h0):
        cols = pl.ds(h0 * dh, GROUP * dh)
        state["q", h0] = _tiles((_matmul(lhs, _bf16(wq[:, cols])) - mean * wq_sum[:, cols]).astype(BF16))

    def mxu_keys(h0, j):
        s = _matmul(state["q", h0][j], _bf16(keys_t[h0 + j]))
        state["s", h0] = s if j == 0 else jnp.where(row_w == j, s, state["s", h0])
        if j == GROUP - 1:
            p, norm = softmax(state["s", h0])
            state["p", h0] = (p.astype(BF16), norm)

    def mxu_values(h0, j):
        p, norm = state["p", h0]
        state["o", h0 + j] = jnp.where(row_d == j, _matmul(p, _bf16(values[h0 + j - vec_heads])) * norm, 0.0).astype(BF16)

    def mxu_output(h0):
        for h in range(h0, h0 + GROUP, 4):
            o = jnp.concatenate([state["o", i] for i in range(h, h + 4)], axis=1)
            _accumulate(mxu_out, 0, _matmul(o, _bf16(wo[pl.ds(h * dh // 2, 4 * dh // 2), :])))

    stages = (lambda h0: [(40 * GROUP, lambda: mxu_query(h0))],
              lambda h0: [(64, lambda j=j: mxu_keys(h0, j)) for j in range(GROUP)],
              lambda h0: [(64, lambda j=j: mxu_values(h0, j)) for j in range(GROUP)],
              lambda h0: [(40 * GROUP, lambda: mxu_output(h0))])
    starts = list(range(vec_heads, heads, GROUP))
    mxu_work = []
    for i in range(len(starts) + len(stages) - 1):
        for lag, stage in enumerate(stages):
            if 0 <= i - lag < len(starts):
                mxu_work += stage(starts[i - lag])

    paced_x = _Paced(_tiles(x), results)
    slot = jnp.where((lane & (GROUP - 1)) == row_d, lane >> 3, -1)

    def vec_keys(g, i):
        if i == 0:
            state["vs", g] = [None] * n_w
        rows = pl.ds(g * GROUP * dh + GROUP * i, GROUP)
        xs = paced_x.get(*PACE_KEYS)
        q = _lane_sum(_sum([vec_qk[t, rows, :] * xs[t] for t in range(n_x)], pairwise=True))
        for t in range(n_w):
            _accumulate(state["vs", g], t, vec_qk[n_x + t, rows, :] * q)
        results.append(state["vs", g][2])
        if i == dh - 1:
            p, norm = softmax(jnp.concatenate(state["vs", g], axis=1))
            state["vp", g] = _Paced(_tiles(p * norm), results)

    def vec_values(g, i):
        rows = pl.ds(g * GROUP * dh + GROUP * i, GROUP)
        moved = g == 0 and i < 16 * MOVED
        ps = state["vp", g].get(*(PACE_MOVED if moved else PACE_VALUES[g]))
        o = _lane_sum(_sum([vec_vo[t, rows, :] * ps[t] for t in range(n_w)]))
        if moved:
            state["lhs"] = jnp.where(slot == i % 16, o, 0.0 if i % 16 == 0 else state["lhs"])
            results.append(state["lhs"])
            if i % 16 == 15:
                w = moved_wo[pl.ds(64 * (i // 16), 64), :]
                _accumulate(mxu_out, 0, _matmul(state["lhs"].astype(BF16), _bf16(w)))
        else:
            for t in range(n_x):
                _accumulate(vec_out, t, vec_vo[n_w + t, rows, :] * o)
            results.append(vec_out[2])

    cost, k = 7.8, 96
    spans = ((vec_keys, 0, 0, dh), (vec_keys, 1, 0, k), (vec_values, 0, 0, dh - k),
             (vec_keys, 1, k, dh), (vec_values, 0, dh - k, dh), (vec_values, 1, 0, dh))
    _interleave(mxu_work, [(cost, lambda fn=fn, g=g, i=i: fn(g, i)) for fn, g, lo, hi in spans for i in range(lo, hi)])
    return x + _row_sum(mxu_out[0] + jnp.concatenate(vec_out, axis=1))


def _make_kernel(batch, heads, seq, window):
    dh = LANES
    n_groups, n_chunks, half = heads // GROUP, window // ROWS, GROUP // 2
    vec_heads = 2 * GROUP
    last = batch - 1
    last_slot = last % 2
    exp_scale = dh ** -0.5 * LOG2E

    def kernel(x_hbm, k_hbm, v_hbm, wq_hbm, wo_hbm, w1t_hbm, b1_hbm, w2_hbm, b2_hbm, o_hbm,
               kbuf, vbuf, wq_in, wo_in, w1t_in, w2_in, x_in, b1_in, b2_in, out,
               wq, wo, w1, w2, wq_sum, w1_sum, b1, b2, xs, qs, acc, p_last, l_last,
               keys_t, values, vec_qk, vec_vo, moved_wo, vec_w, vec_b1,
               kv_sem, last_sem, w_sem):
        d, ff = xs.shape[1], b1_in.shape[0]
        n_x, n_w = d // LANES, window // LANES

        def kv_copy(src, dst, src_head, slot, head, row, sem):
            return pltpu.make_async_copy(src.at[pl.ds(src_head, PAIR), pl.ds(seq - window + row, ROWS), :],
                                         dst.at[slot, pl.ds(head, PAIR), pl.ds(row, ROWS), :], sem)

        def start_group(n, lo, hi):
            if isinstance(n, int):
                slot, g = (n // n_groups) % 2, n % n_groups
            else:
                slot, g = lax.shift_right_logical(n, n_groups.bit_length() - 1) & 1, n & (n_groups - 1)

            def chunk(i):
                row = _times(i, ROWS)
                for h in range(0, GROUP, PAIR):
                    kv_copy(k_hbm, kbuf, n * GROUP + h, slot, g * GROUP + h, row, kv_sem.at[0, slot, g]).start(priority=0)
                    kv_copy(v_hbm, vbuf, n * GROUP + h, slot, g * GROUP + h, row, kv_sem.at[1, slot, g]).start(priority=1)
            _loop(lo, hi, chunk)

        def start_after(n, lo, hi):
            for k in range(2):
                start_group(n + 1 + k, max(lo - k * n_chunks, 0), min(hi - k * n_chunks, n_chunks))

        def wait(region, sem):
            pltpu.make_async_copy(region, region, sem).wait()

        def wait_group(slot, g):
            wait(kbuf.at[slot, pl.ds(g * GROUP, GROUP)], kv_sem.at[0, slot, g])
            wait(vbuf.at[slot, pl.ds(g * GROUP, GROUP)], kv_sem.at[1, slot, g])

        parts = [(src, dst, g * GROUP) for src, dst in ((k_hbm, kbuf), (v_hbm, vbuf)) for g in range(n_groups)]
        per_chunk = GROUP // PAIR
        per_part = n_chunks * per_chunk
        end_rows = window // 4
        pieces = [(heads - 2 * GROUP, half, 0, window), (heads - GROUP - half, half, 0, window),
                  (heads - GROUP, half, 0, window), (heads - half, PAIR, 0, window),
                  (heads - PAIR, PAIR, 0, window - end_rows), (heads - PAIR, PAIR, window - end_rows, end_rows)]
        started = [0]

        def piece_sem(n):
            return last_sem.at[len(parts) - 2 + n]

        def start_last(upto):
            for i, (src, dst, h0) in enumerate(parts):
                lo, hi = (min(max((e - i * per_part) // per_chunk, 0), n_chunks) for e in (started[0], upto))
                whole = i < len(parts) - 2
                sem0 = last_sem.at[i] if whole else piece_sem(2 * (i - len(parts) + 2))
                sem1 = last_sem.at[i] if whole else piece_sem(1)

                def chunk(k, late=None, src=src, dst=dst, h0=h0, sem0=sem0, sem1=sem1):
                    for j, h in enumerate(range(h0, h0 + half, PAIR)):
                        kv_copy(src, dst, last * heads + h, last_slot, h, _times(k, ROWS), sem0).start(priority=0)
                        if late is None:
                            h1, c, sem = h + half, k, sem1
                        else:
                            h1, c, sem = late[0], 2 * (k - late[1]) + j, late[2]
                        kv_copy(src, dst, last * heads + h1, last_slot, h1, _times(c, ROWS), sem).start(priority=1)

                if i < len(parts) - 1:
                    _loop(lo, hi, chunk)
                    continue
                for n, (h1, _, r0, nr) in list(enumerate(pieces))[3:]:
                    k0 = (h1 - (heads - half)) // PAIR * (n_chunks // 2)
                    a, b = k0 + r0 // (2 * ROWS), k0 + (r0 + nr) // (2 * ROWS)
                    _loop(max(lo, a), min(hi, b), lambda k, late=(h1, k0, piece_sem(n)): chunk(k, late))
            started[0] = max(started[0], upto)

        def receive_last(i):
            _, dst, h0 = parts[i]
            start_last((i + 1) * per_part + LEAD)
            wait(dst.at[last_slot, pl.ds(h0, GROUP)], last_sem.at[i])

        def start_weights(src0, dst0, sem0, cols, src1, dst1, sem1):
            n0, ratio = src0.shape[1] // 8, src1.shape[1] // src0.shape[1]

            def strip(i):
                rows0 = pl.ds(_times(i, 8), 8)
                for k in range(ratio):
                    cols0, rows1 = pl.ds(k * cols, cols), pl.ds(_times(i * ratio + k, 8), 8)
                    pltpu.make_async_copy(src0.at[:, rows0, cols0], dst0.at[:, rows0, cols0], sem0).start(priority=0)
                    pltpu.make_async_copy(src1.at[:, rows1], dst1.at[:, rows1], sem1).start(priority=1)
            _loop(0, n0, strip)

        def repack(src, dst):
            n = src.shape[1] // 2

            def part(i):
                dst[pl.ds(_times(i, n), n), :] = pltpu.bitcast(src[i], U32)
            _loop(0, src.shape[0], part)

        row_w = lax.broadcasted_iota(jnp.int32, (8, window), 0)
        row_d = lax.broadcasted_iota(jnp.int32, (8, dh), 0)
        row_x = lax.broadcasted_iota(jnp.int32, (8, d), 0)

        small = [pltpu.make_async_copy(src, dst, w_sem.at[i])
                 for i, (src, dst) in enumerate(((x_hbm, x_in), (b1_hbm, b1_in), (b2_hbm, b2_in)))]
        for copy in small:
            copy.start()
        start_weights(wq_hbm, wq_in, w_sem.at[3], 512, wo_hbm, wo_in, w_sem.at[4])
        start_weights(w1t_hbm, w1t_in, w_sem.at[5], d, w2_hbm, w2_in, w_sem.at[6])

        small[0].wait()
        x0 = x_in[...].astype(F32)
        xs[...] = x0
        acc[...] = jnp.zeros_like(acc)
        wait(wq_in, w_sem.at[3])
        repack(wq_in, wq)
        start_group(0, 0, n_chunks // 2)
        q0 = _matmul(jnp.concatenate([_layernorm(x0), jnp.ones((8, d), F32)], axis=0).astype(BF16), _bf16(wq[...]))
        qs[...] = q0[:8]
        wq_sum[...] = q0[8:]
        start_group(0, n_chunks // 2, n_chunks)
        wait(wo_in, w_sem.at[4])
        repack(wo_in, wo)
        start_group(1, 0, AHEAD // 2)
        small[1].wait()
        small[2].wait()
        wait(w1t_in, w_sem.at[5])
        wait(w2_in, w_sem.at[6])
        repack(w2_in, w2)
        w1t = w1t_in[...].reshape(ff, d)
        for f in range(0, ff, LANES):
            rows = w1t[f:f + LANES]
            if rows.shape[0] < LANES:
                rows = jnp.concatenate([rows, jnp.zeros((LANES - rows.shape[0], d), BF16)], axis=0)
            w1[:, pl.ds(f, LANES)] = pltpu.bitcast(rows.T, U32)
        w1_sum[...] = _matmul(jnp.ones((8, d), BF16), _bf16(w1[...]))
        bias = b1_in[...].astype(F32).reshape(1, ff)
        bias = jnp.concatenate([bias, jnp.zeros((1, b1.shape[1] - ff), F32)], axis=1)
        b1[...] = jnp.broadcast_to(bias, b1.shape)
        b2[...] = jnp.broadcast_to(b2_in[...].astype(F32).reshape(1, d), b2.shape)
        start_group(1, AHEAD // 2, AHEAD)

        def probs(h, prev, cur):
            q = qs[:, pl.ds(_times(h, dh), dh)].astype(BF16)
            s = None
            if prev is not None:
                s = _matmul(q, _bf16(keys_t[h]))
            if cur is not None:
                fresh = lax.dot_general(q, kbuf[cur[1], h], (((1,), (1,)), ((), ())), preferred_element_type=F32)
                s = fresh if s is None else jnp.where(row_w == cur[0], fresh, s)
            p = jnp.exp2((s - jnp.max(s, axis=-1, keepdims=True)) * exp_scale)
            return p.astype(BF16), jnp.sum(p, axis=-1, keepdims=True)

        def keep_keys(h, slot):
            keys_t[h] = pltpu.bitcast(kbuf[slot, h].T, U32)

        def project(h0, rows, weights):
            outs = []
            for j, (p, total) in enumerate(weights):
                o, norm = jnp.zeros((8, dh), F32), 1.0 / total
                for row, slot in rows:
                    o = jnp.where(row_d == row, _matmul(p, vbuf[slot, h0 + j]) * norm, o)
                outs.append(o.astype(BF16))
            w = wo[pl.ds(_times(h0, dh // 2), len(weights) * dh // 2), :]
            acc[...] += _matmul(jnp.concatenate(outs, axis=-1), _bf16(w))

        def mlp(active):
            x1 = xs[...] + acc[...]
            h = _gelu(_matmul(_layernorm(x1).astype(BF16), _bf16(w1[...])) + b1[...])[:, :ff]
            x2 = jnp.where(active, x1 + _matmul(h.astype(BF16), _bf16(w2[...])) + b2[...], xs[...])
            xs[...] = x2
            acc[...] = jnp.where(active, 0.0, acc[...])
            return x2

        def queries(x):
            qs[...] = _matmul(_layernorm(x).astype(BF16), _bf16(wq[...]))

        marks = [AHEAD + STEP * i for i in range(5)]

        def group(b, g, prev, start, extra=None):
            slot = b & 1
            wait_group(slot, g)
            rows = ([] if prev is None else [(prev, 1 - slot)]) + [(b, slot)]
            for i in range(2):
                h0 = g * GROUP + i * half
                weights = [probs(h0 + j, prev, (b, slot)) for j in range(half)]
                for j in range(half):
                    keep_keys(h0 + j, slot)
                start(2 * i)
                project(h0, rows, weights)
                if extra is not None:
                    extra(i)
                start(2 * i + 1)

        def whole_batch(b, prev, extra):
            def body(g):
                n = b * n_groups + g
                group(b, g, prev, lambda i: start_after(n, marks[i], marks[i + 1]), lambda i: extra(2 * g + i))
                pl.when(g < n_groups - 1)(lambda: start_after(n, marks[-1], n_chunks + AHEAD))
            _loop(0, n_groups, body)
            n = b * n_groups + n_groups - 1
            x = mlp(row_x == b if prev is None else (row_x == b) | (row_x == prev))
            start_after(n, marks[-1], marks[-1] + MID)
            queries(x)
            start_after(n, marks[-1] + MID, n_chunks + AHEAD)

        def spread(dst, first_tile, h, value):
            g, j = divmod(h, GROUP) if isinstance(h, int) else (lax.shift_right_logical(h, 3), h & (GROUP - 1))
            for t, tile in enumerate(_tiles(value)):
                dst[first_tile + t, pl.ds(g * (GROUP * dh) + j, dh, stride=GROUP), :] = tile

        def prepare_heads(k):
            n = vec_heads * half // heads
            for j in range(n):
                h = k * n + j
                cols = _bf16(wq[:, pl.ds(_times(h, dh), dh)]).T.astype(F32)
                spread(vec_qk, 0, h, cols - jnp.mean(cols, axis=-1, keepdims=True))
                spread(vec_vo, n_w, h, _bf16(wo[pl.ds(_times(h, dh // 2), dh // 2), :]).astype(F32))

        def prepare_hidden(k, n):
            f = _times(MXU_FF // LANES + k, LANES)
            up = _bf16(w1[:, pl.ds(f, LANES)]).T.astype(F32)[:n]
            down = _bf16(w2[pl.ds(_times(MXU_FF // LANES + k, LANES // 2), n // 2), :]).astype(F32)
            rows = pl.ds(_times(k, LANES), n)
            vec_w[rows, :] = jnp.concatenate([up - jnp.mean(up, axis=-1, keepdims=True), down], axis=1)
            vec_b1[rows, :] = jnp.broadcast_to(b1[0:1, pl.ds(f, LANES)], (LANES, LANES)).T[:n]

        def prepare_moved(i):
            rows = [vec_vo[n_w + t, pl.ds(_times(i, LANES), LANES), :] for t in range(n_x)]
            moved_wo[pl.ds(_times(i, 64), 64), :] = pltpu.bitcast(jnp.concatenate(rows, axis=1).astype(BF16), U32)

        whole_batch(0, None, prepare_heads)

        def step(b):
            def extra(k):
                full, rest = divmod(vec_w.shape[0], LANES)

                @pl.when(b == 1)
                def _():
                    pl.when(k < full)(lambda: prepare_hidden(k, LANES))
                    if rest:
                        pl.when(k == full)(lambda: prepare_hidden(full, rest))
                    pl.when(k < MOVED)(lambda: prepare_moved(k))
            whole_batch(b, b - 1, extra)
        _loop(1, last - 1, step)

        b = last - 1
        slot = b % 2

        def body(g):
            n = b * n_groups + g
            group(b, g, b - 1, lambda i: start_after(n, marks[i], marks[i + 1] if i < 3 else n_chunks + AHEAD))
        _loop(0, n_groups - 2, body)

        def start(i):
            start_group(last * n_groups - 1, min(marks[i], n_chunks), min(marks[i + 1], n_chunks))
            start_last(2 * per_chunk * max(marks[i + 1] - n_chunks, 0))
        group(b, n_groups - 2, b - 1, start)

        h0 = heads - GROUP
        project(h0, [(b - 1, 1 - slot)], [probs(h0 + j, b - 1, None) for j in range(GROUP)])
        start_last(LEAD)
        wait_group(slot, n_groups - 1)
        weights = [probs(h0 + j, None, (b, slot)) for j in range(GROUP)]
        for j in range(GROUP):
            keep_keys(h0 + j, slot)
        project(h0, [(b, slot)], weights)
        start_last(LAST_MARKS[0])
        x = mlp((row_x == b) | (row_x == b - 1))
        start_last(LAST_MARKS[1])
        queries(x)
        start_last(LAST_MARKS[2])

        for g in range(n_groups):
            receive_last(g)
            h0 = g * GROUP
            weights = [probs(h0 + j, last - 1, (last, last_slot)) for j in range(GROUP)]
            project(h0, [(last - 1, 1 - last_slot)], weights)
            for h, (p, total) in enumerate(weights, h0):
                p_last[h] = jnp.broadcast_to(p.astype(F32)[last:last + 1], (8, window))
                l_last[h] = jnp.broadcast_to(total[last:last + 1], (8, dh))
                if h < vec_heads:
                    spread(vec_qk, n_x, h, kbuf[last_slot, h].T.astype(F32))
                else:
                    keep_keys(h, last_slot)
            start_last(LAST_MARKS[3 + g])
        mlp(row_x == last - 1)
        for g in range(vec_heads // GROUP):
            receive_last(n_groups + g)
            hs = range(g * GROUP, (g + 1) * GROUP)
            project(g * GROUP, [(last, last_slot)], [(p_last[h].astype(BF16), l_last[h]) for h in hs])
            for h in hs:
                spread(vec_vo, 0, h, vbuf[last_slot, h].T.astype(F32))
        start_last(len(parts) * per_part)

        partial = {}
        x = jnp.broadcast_to((xs[...] + acc[...])[last:last + 1], (8, d))
        for n, (h0, nh, r0, nr) in enumerate(pieces):
            wait(vbuf.at[last_slot, pl.ds(h0, nh), pl.ds(r0, nr)], piece_sem(n))
            for h in range(h0, h0 + nh):
                v = vbuf[last_slot, h, pl.ds(r0, nr), :]
                values[h - vec_heads, pl.ds(r0 // 2, nr // 2), :] = pltpu.bitcast(v, U32)
                o = _matmul(p_last[h, :, pl.ds(r0, nr)].astype(BF16), v)
                partial[h] = o + partial[h] if r0 else o
            if r0 + nr == window:
                o = jnp.concatenate([partial[h] * (1.0 / l_last[h]) for h in range(h0, h0 + nh)], axis=-1).astype(BF16)
                x = x + _matmul(o, _bf16(wo[pl.ds(h0 * dh // 2, nh * dh // 2), :]))

        x = _row_mlp(x, w1, w2, b1, b2, w1_sum, vec_w, vec_b1)
        x = _row_attention(x, exp_scale, wq, wq_sum, wo, keys_t, values,
                           vec_qk, vec_vo, moved_wo, vec_heads, heads)
        x = _row_mlp(x, w1, w2, b1, b2, w1_sum, vec_w, vec_b1)
        out[...] = jnp.where(row_x == last, x, xs[...]).astype(out.dtype)
        copy = pltpu.make_async_copy(out, o_hbm, w_sem.at[0])
        copy.start()
        copy.wait()

    return kernel


def _run(x, k_cache, v_cache, wq, wo, w1, b1, w2, b2):
    batch, _, d = x.shape
    _, heads, seq, dh = k_cache.shape
    window = min(4096, max(256, seq // 4))
    ff, e = w1.shape[1], heads * dh
    ff_padded = pl.cdiv(ff, LANES) * LANES
    assert (batch, heads, window, dh) == (8, 4 * GROUP, 16 * ROWS, LANES) and d % LANES == 0
    wq, wo = wq.reshape(5, d // 5, e), wo.reshape(4, e // 4, d)
    w1t, w2 = w1.T.reshape(4, ff // 4, d), w2.reshape(4, ff // 4, d)
    vec_ff = ff - MXU_FF
    vec_rows = 2 * GROUP * dh + 8

    vmem, dma, hbm = pltpu.VMEM, pltpu.SemaphoreType.DMA, pl.BlockSpec(memory_space=pltpu.HBM)
    out = pl.pallas_call(
        _make_kernel(batch, heads, seq, window),
        out_shape=jax.ShapeDtypeStruct((batch, d), x.dtype),
        in_specs=[hbm] * 9,
        out_specs=hbm,
        scratch_shapes=[
            vmem((2, heads, window, dh), BF16), vmem((2, heads, window, dh), BF16),
            vmem(wq.shape, BF16), vmem(wo.shape, BF16), vmem(w1t.shape, BF16), vmem(w2.shape, BF16),
            vmem((batch, d), BF16), vmem((ff,), BF16), vmem((d,), BF16), vmem((batch, d), x.dtype),
            vmem((d // 2, e), U32), vmem((e // 2, d), U32), vmem((d // 2, ff_padded), U32), vmem((ff // 2, d), U32),
            vmem((8, e), F32), vmem((8, ff_padded), F32), vmem((8, ff_padded), F32), vmem((8, d), F32),
            vmem((batch, d), F32), vmem((batch, e), F32), vmem((batch, d), F32),
            vmem((heads, 8, window), F32), vmem((heads, 8, dh), F32),
            vmem((heads, dh // 2, window), U32), vmem((heads - 2 * GROUP, window // 2, dh), U32),
            vmem(((d + window) // LANES, vec_rows, LANES), F32), vmem(((d + window) // LANES, vec_rows, LANES), F32),
            vmem((64 * MOVED, d), U32), vmem((vec_ff, 2 * d), F32), vmem((vec_ff, LANES), F32),
            dma((2, 2, heads // GROUP)), dma((2 * heads // GROUP + 4,)), dma((7,)),
        ],
        compiler_params=pltpu.CompilerParams(vmem_limit_bytes=124 * 2**20, disable_bounds_checks=True,
                                             disable_semaphore_checks=True),
    )(x.reshape(batch, d), k_cache.reshape(batch * heads, seq, dh), v_cache.reshape(batch * heads, seq, dh),
      wq, wo, w1t, b1, w2, b2)
    return out.reshape(batch, 1, d)


@jax.jit
def pallas_interleave_layers__sliding_block_cached__mixer_channel_mlp__decode_kernel(
    A_x: jax.Array,
    A_k_cache: jax.Array,
    A_v_cache: jax.Array,
    A_wq: jax.Array,
    A_wo: jax.Array,
    B_x: jax.Array,
    B_w1: jax.Array,
    B_b1: jax.Array,
    B_w2: jax.Array,
    B_b2: jax.Array,
):
    del B_x
    return _run(A_x, A_k_cache, A_v_cache, A_wq, A_wo, B_w1, B_b1, B_w2, B_b2)
```
